```python
import jax
import jax.numpy as jnp

def _softmax(x, axis=-1):
    return jax.nn.softmax(x, axis=axis)

def _gelu(x):
    return jax.nn.gelu(x, approximate=True)

def _silu(x):
    return jax.nn.silu(x)

def _sigmoid(x):
    return jax.nn.sigmoid(x)

def _layernorm(x, axis=-1, eps=1e-05):
    m = jnp.mean(x, axis=axis, keepdims=True)
    v = jnp.var(x, axis=axis, keepdims=True)
    return (x - m) / jnp.sqrt(v + eps)

def _scatter_add(tgt, idx, src, axis=0):
    return tgt.at[idx].add(src)

def _segment_sum(src, seg, n):
    return jax.ops.segment_sum(src, seg, n)

class _Rng:

    def __init__(self, key):
        self._k = key

    def _next(self):
        self._k, sub = jax.random.split(self._k)
        return sub

    def normal(self, shape):
        return jax.random.normal(self._next(), shape, dtype=jnp.bfloat16)

    def randint(self, lo, hi, shape):
        return jax.random.randint(self._next(), shape, lo, hi, dtype=jnp.int32)

    def uniform(self, shape, lo=0.0, hi=1.0):
        return jax.random.uniform(self._next(), shape, jnp.bfloat16, lo, hi)

    def permutation(self, n):
        return jax.random.permutation(self._next(), n)
kernel_name = 'interleave_layers__memory_aug_infini_attn__sliding_local_dilated__prompt'

def setup_inputs():
    _rng = _Rng(jax.random.key(int.from_bytes(__import__("os").urandom(4), "little")))
    _w = lambda a: (lambda t: t.astype(jnp.bfloat16) if jnp.issubdtype(t.dtype, jnp.floating) else t)(jnp.asarray(a))

    def _A_setup():
        B, S, D, H = (1, 2048, 1024, 32)
        N = 4
        L = max(1, S // N)
        sc = D ** (-0.5)
        return {'x': _w((lambda *s: _rng.normal(s) * 0.05)(B, N * L, D)), 'wq': _w((lambda *s: _rng.normal(s) * 0.05)(D, D) * sc), 'wk': _w((lambda *s: _rng.normal(s) * 0.05)(D, D) * sc), 'wv': _w((lambda *s: _rng.normal(s) * 0.05)(D, D) * sc), 'wo': _w((lambda *s: _rng.normal(s) * 0.05)(D, D) * sc), 'beta': _w((lambda *s: _rng.normal(s) * 0.05)(H))}
    _A_in = _A_setup()

    def _B_setup():
        B, S, D = (1, 2048, 1024)
        return {'x': _w((lambda *s: _rng.normal(s) * 0.05)(B, S, D)), 'wqkv': _w((lambda *s: _rng.normal(s) * 0.05)(D, 3 * D)), 'wo': _w((lambda *s: _rng.normal(s) * 0.05)(D, D))}
    _B_in = _B_setup()
    return {'A_x': _A_in['x'], 'A_wq': _A_in['wq'], 'A_wk': _A_in['wk'], 'A_wv': _A_in['wv'], 'A_wo': _A_in['wo'], 'A_beta': _A_in['beta'], 'B_x': _B_in['x'], 'B_wqkv': _B_in['wqkv'], 'B_wo': _B_in['wo']}

def reference(A_x, A_wq, A_wk, A_wv, A_wo, A_beta, B_x, B_wqkv, B_wo):

    def _A_ref(x, wq, wk, wv, wo, beta):
        B, S, D = x.shape
        H = 32
        Dh = D // H
        N = 4
        L = S // N
        q = (lambda x, *d: x.transpose(*d))((x @ wq).reshape(B, S, H, Dh), 0, 2, 1, 3).reshape(B, H, N, L, Dh)
        k = (lambda x, *d: x.transpose(*d))((x @ wk).reshape(B, S, H, Dh), 0, 2, 1, 3).reshape(B, H, N, L, Dh)
        v = (lambda x, *d: x.transpose(*d))((x @ wv).reshape(B, S, H, Dh), 0, 2, 1, 3).reshape(B, H, N, L, Dh)
        phi = lambda t: jnp.where(t > 0, t + 1.0, jnp.exp(t))
        scale = Dh ** (-0.5)
        ar = jnp.arange(L)
        mask = (lambda x, dt: x.astype(dt))(ar[:, None] < ar[None, :], x.dtype) * -1000000000.0
        g = _sigmoid(beta).reshape(1, H, 1, 1)
        M = jnp.einsum('bhd,bhe->bhde', q[:, :, 0, 0, :] * 0.0, q[:, :, 0, 0, :] * 0.0)
        z = q[:, :, 0, 0, :] * 0.0
        outs = []
        for s in range(N):
            qs, ks, vs = (q[:, :, s].copy(), k[:, :, s].copy(), v[:, :, s].copy())
            logits = jnp.einsum('bhqd,bhkd->bhqk', qs, ks) * scale + mask
            p = _softmax(logits, axis=-1)
            a_dot = jnp.einsum('bhqk,bhkd->bhqd', p, vs)
            pq = phi(qs)
            num = jnp.einsum('bhld,bhde->bhle', pq, M)
            den = jnp.einsum('bhld,bhd->bhl', pq, z)[..., None] + 1e-06
            a_mem = num / den
            o = g * a_mem + (1.0 - g) * a_dot
            outs.append(o)
            pk = phi(ks)
            M = M + jnp.einsum('bhld,bhle->bhde', pk, vs)
            z = z + jnp.einsum('bhld->bhd', pk)
        o = (lambda x, *d: x.transpose(*d))(jnp.stack(outs, 2).reshape(B, H, S, Dh), 0, 2, 1, 3).reshape(B, S, D)
        return o @ wo

    def _B_ref(x, wqkv, wo):
        B, S, D = x.shape
        H = 32
        Dh = D // H
        W, dil = (8, 2)
        qkv = (lambda x, *d: x.transpose(*d))((x @ wqkv).reshape(B, S, 3, H, Dh), 2, 0, 3, 1, 4)
        q, k, v = (qkv[0], qkv[1], qkv[2])
        scale = Dh ** (-0.5)
        pos = jnp.arange(S)
        off = jnp.arange(W) * dil
        idx = pos[:, None] - off[None, :]
        mask = idx >= 0
        idx_c = jnp.where(mask, idx, 0).reshape(-1)
        kg = k[:, :, idx_c, :].reshape(B, H, S, W, Dh)
        vg = v[:, :, idx_c, :].reshape(B, H, S, W, Dh)
        logits = jnp.einsum('bhsd,bhswd->bhsw', q, kg) * scale
        logits = jnp.where(mask[None, None, :, :], logits, -1000000000.0)
        attn = _softmax(logits, axis=-1)
        o = jnp.einsum('bhsw,bhswd->bhsd', attn, vg)
        return (lambda x, *d: x.transpose(*d))(o, 0, 2, 1, 3).reshape(B, S, D) @ wo
    x = A_x
    x = x + _A_ref(_layernorm(x, axis=-1), A_wq, A_wk, A_wv, A_wo, A_beta)
    x = x + _B_ref(_layernorm(x, axis=-1), B_wqkv, B_wo)
    x = x + _A_ref(_layernorm(x, axis=-1), A_wq, A_wk, A_wv, A_wo, A_beta)
    x = x + _B_ref(_layernorm(x, axis=-1), B_wqkv, B_wo)
    return x
```

```python
import math

import jax
import jax.numpy as jnp
from jax import lax
import jax.experimental.pallas as pl
import jax.experimental.pallas.tpu as pltpu

S = 2048
D = 1024
H = 32
DH = D // H
NSEG = 4
L = S // NSEG
WIN, DIL = 8, 2
HALO = 16
G = D // 128
CH = 128
NCH = L // CH
LOG2E = math.log2(math.e)
QSCALE = DH ** -0.5 * LOG2E
NEG = -1e9

F32, BF16, U32 = jnp.float32, jnp.bfloat16, jnp.uint32
NN = (((1,), (0,)), ((), ()))
NT = (((1,), (1,)), ((), ()))


def _dot(a, b, dims=NN):
    return lax.dot_general(a, b, dims, preferred_element_type=F32)


def _pack(x):
    return pltpu.bitcast(x.astype(BF16), U32)


def _unpack(x):
    return pltpu.bitcast(x, BF16)


def _layernorm(x):
    m = jnp.mean(x, axis=-1, keepdims=True)
    d = x - m
    v = jnp.mean(d * d, axis=-1, keepdims=True)
    return d * lax.rsqrt(v + 1e-5)


def _phi(t):
    return jnp.where(t > 0, t + 1.0, jnp.exp(t))


def _iota(shape, dim):
    return lax.broadcasted_iota(jnp.int32, shape, dim)


def _kernel(x_hbm, wq_hbm, wk_hbm, wv_hbm, wo_hbm, beta_ref, wqkv_hbm, wob_hbm, out_hbm,
            xin, wq, wk, wv, wo, wqkv_raw, wob_raw, wbt, wob, tmp, xres, hbuf, obuf, ostage,
            mem, zmem, gate, qb, kb, vb, ktail, vtail, sems, osem):
    def x_copy(s):
        return pltpu.make_async_copy(x_hbm.at[pl.ds(s * L, L)], xin.at[s], sems.at[s])

    w_copies = [
        pltpu.make_async_copy(src, dst, sems.at[NSEG + i])
        for i, (src, dst) in enumerate(
            [(wq_hbm, wq), (wk_hbm, wk), (wv_hbm, wv), (wo_hbm, wo), (wqkv_hbm, wqkv_raw), (wob_hbm, wob_raw)])
    ]
    x_copy(0).start()
    for c in w_copies:
        c.start()
    for s in range(1, NSEG):
        x_copy(s).start()

    b = beta_ref[...].astype(F32).reshape(1, H)
    b = jnp.where(_iota((H, H), 0) == _iota((H, H), 1), jnp.broadcast_to(b, (H, H)), 0.0)
    b = jnp.sum(b, axis=1, keepdims=True)
    gate[...] = jnp.broadcast_to(1.0 / (1.0 + jnp.exp(-b)), (H, 128))
    mem[...] = jnp.zeros(mem.shape, F32)
    zmem[...] = jnp.zeros(zmem.shape, F32)
    ktail[...] = jnp.zeros(ktail.shape, F32)
    vtail[...] = jnp.zeros(vtail.shape, F32)

    x_copy(0).wait()
    for c in range(NCH):
        x0 = xin[0, pl.ds(c * CH, CH), :].astype(F32)
        xres[pl.ds(c * CH, CH), :] = x0
        hbuf[pl.ds(c * CH // 2, CH // 2), :] = _pack(_layernorm(x0))
    for c in w_copies[:4]:
        c.wait()

    def permute_rows(dst, base):
        for e in range(DH // 2):
            w = jnp.concatenate([tmp[j, pl.ds(e, H, stride=DH // 2), :] for j in range(G)], axis=1)
            lo = lax.bitcast_convert_type(w << 16, F32)
            hi = lax.bitcast_convert_type(w & jnp.uint32(0xFFFF0000), F32)
            dst[pl.ds(base + e * H, H), :] = _pack(jnp.concatenate([lo, hi], axis=0))

    def prepare_b_weights():
        w_copies[4].wait()
        w_copies[5].wait()
        for s in range(1, NSEG):
            x_copy(s).wait()

        def one(i, carry):
            col = pl.multiple_of(i * D, D)
            for j in range(G):
                tmp[j] = pltpu.bitcast(wqkv_raw[pl.ds(j * 128, 128), pl.ds(col, D)].T, U32)
            permute_rows(wbt, pl.multiple_of(i * (D // 2), D // 2))
            return carry

        lax.fori_loop(0, 3, one, 0)
        for j in range(G):
            tmp[j] = pltpu.bitcast(wob_raw[:, pl.ds(j * 128, 128)], U32)
        permute_rows(wob, 0)

    def a_proj(g):
        h = _unpack(hbuf[...])
        cols = pl.ds(g * 128, 128)
        return _dot(h, wq[:, cols]), _dot(h, wk[:, cols]), _dot(h, wv[:, cols])

    def a_attn(g, pair, q, k, v):
        qs = (q * QSCALE).astype(BF16)
        kk = k.astype(BF16)
        vt = v.astype(BF16).T
        pq = _phi(q).astype(BF16)
        pk = _phi(k)

        m_old = mem[pair, g]
        z_old = zmem[pair, g]
        r = _dot(jnp.concatenate([m_old, z_old], axis=0).astype(BF16), pq, NT)
        same = _iota((128, 128), 0) // DH == _iota((128, 128), 1) // DH
        mem[pair, g] = m_old + jnp.where(same, _dot(vt, pk.astype(BF16)), 0.0)
        zsel = _iota((16, 128), 0) == _iota((16, 128), 1) // DH
        zmem[pair, g] = z_old + jnp.where(zsel, jnp.sum(pk, axis=0, keepdims=True), 0.0)
        rden = 1.0 / (r[128:136] + 1e-6)

        lane_head = _iota((CH, 128), 1) // DH
        causal = _iota((CH, CH), 0) <= _iota((CH, CH), 1)
        cols = []
        for j in range(NCH):
            n = (j + 1) * CH
            qj = qs[j * CH:n]
            rows = []
            for hh in range(4):
                st = _dot(kk[:n], jnp.where(lane_head == hh, qj, jnp.zeros_like(qj)), NT)
                diag = jnp.where(causal, st[n - CH:], NEG)
                st = diag if j == 0 else jnp.concatenate([st[:n - CH], diag], axis=0)
                p = jnp.exp2(st - jnp.max(st, axis=0, keepdims=True))
                l = jnp.sum(p, axis=0, keepdims=True)
                o = _dot(vt[hh * DH:(hh + 1) * DH, :n], p.astype(BF16))
                gt = gate[pl.ds(4 * g + hh, 1), :]
                rows.append(o * ((1.0 - gt) / l)
                            + r[hh * DH:(hh + 1) * DH, j * CH:n] * (gt * rden[hh:hh + 1, j * CH:n]))
            cols.append(jnp.concatenate(rows, axis=0).astype(BF16))
        ot = jnp.concatenate(cols, axis=1)
        obuf[:, pl.ds(g * 128, 128)] = pltpu.bitcast(ot.T, U32)

    def a_out(c):
        rows, half = pl.ds(c * CH, CH), pl.ds(c * CH // 2, CH // 2)
        x = xres[rows, :] + _dot(_unpack(obuf[half, :]), wo[...])
        xres[rows, :] = x
        hbuf[half, :] = _pack(_layernorm(x))

    def b_proj(c):
        h = _unpack(hbuf[pl.ds(c * CH // 2, CH // 2), :])
        for i, (dst, off) in enumerate([(qb, 0), (kb, HALO), (vb, HALO)]):
            y = _dot(h, _unpack(wbt[pl.ds(i * D // 2, D // 2), :]), NT)
            if i == 0:
                y = y * QSCALE
            for j in range(G):
                dst[j, pl.ds(off + c * CH, CH), :] = y[:, j * 128:(j + 1) * 128]

    def b_attn(c, seg):
        T = 16
        for t0 in range(c * CH, (c + 1) * CH, T):
            q = [qb[j, pl.ds(t0, T), :] for j in range(G)]
            logits = []
            for w in range(WIN):
                rows = pl.ds(HALO + t0 - DIL * w, T)
                a = q[0] * kb[0, rows, :]
                for j in range(1, G):
                    a = a + q[j] * kb[j, rows, :]
                a = a + pltpu.roll(a, 64, 1)
                a = a + pltpu.roll(a, 32, 1)
                if t0 < DIL * w:
                    a = jnp.where(_iota((T, 128), 0) + (seg * L + t0) >= DIL * w, a, NEG)
                logits.append(a)
            m = logits[0]
            for a in logits[1:]:
                m = jnp.maximum(m, a)
            p = [jnp.exp2(a - m) for a in logits]
            l = p[0]
            for a in p[1:]:
                l = l + a
            rl = 1.0 / l
            outs = []
            for j in range(G):
                o = p[0] * vb[j, pl.ds(HALO + t0, T), :]
                for w in range(1, WIN):
                    o = o + p[w] * vb[j, pl.ds(HALO + t0 - DIL * w, T), :]
                outs.append(o * rl)
            obuf[pl.ds(t0 // 2, T // 2), :] = _pack(jnp.concatenate(outs, axis=1))

    def b_out(c, seg, pair):
        rows, half = pl.ds(c * CH, CH), pl.ds(c * CH // 2, CH // 2)
        x = xres[rows, :] + _dot(_unpack(obuf[half, :]), _unpack(wob[...]))
        ostage[seg, rows, :] = x.astype(BF16)
        nxt = xin[jnp.minimum(seg + 1, NSEG - 1), rows, :].astype(F32)
        x = jnp.where(pair == 1, nxt, x)
        xres[rows, :] = x
        hbuf[half, :] = _pack(_layernorm(x))

    def out_copy(s):
        return pltpu.make_async_copy(ostage.at[s], out_hbm.at[pl.ds(s * L, L)], osem.at[s])

    def step(it, carry):
        seg, pair = it // 2, it % 2
        qkv = a_proj(0)
        for g in range(G):
            nxt = a_proj(g + 1) if g + 1 < G else None
            a_attn(g, pair, *qkv)
            qkv = nxt
        for c in range(NCH):
            a_out(c)

        pl.when(it == 0)(prepare_b_weights)

        kb[:, pl.ds(0, HALO), :] = ktail[pair]
        vb[:, pl.ds(0, HALO), :] = vtail[pair]
        b_proj(0)
        for c in range(NCH):
            if c + 1 < NCH:
                b_proj(c + 1)
            else:
                for cc in range(NCH - 1):
                    b_out(cc, seg, pair)
            b_attn(c, seg)
        b_out(NCH - 1, seg, pair)
        ktail[pair] = kb[:, pl.ds(L, HALO), :]
        vtail[pair] = vb[:, pl.ds(L, HALO), :]

        @pl.when(pair == 1)
        def _():
            out_copy(seg).start()

        return carry

    lax.fori_loop(0, 2 * NSEG, step, 0)
    for s in range(NSEG):
        out_copy(s).wait()


@jax.jit
def pallas_interleave_layers__memory_aug_infini_attn__sliding_local_dilated__prompt_kernel(
    A_x, A_wq, A_wk, A_wv, A_wo, A_beta, B_x, B_wqkv, B_wo,
):
    del B_x
    hbm = pl.BlockSpec(memory_space=pl.ANY)
    vm = pltpu.VMEM
    out = pl.pallas_call(
        _kernel,
        name="infini_dilated",
        out_shape=jax.ShapeDtypeStruct((S, D), BF16),
        in_specs=[hbm, hbm, hbm, hbm, hbm, pl.BlockSpec(memory_space=pltpu.VMEM), hbm, hbm],
        out_specs=hbm,
        scratch_shapes=[
            vm((NSEG, L, D), BF16),
            vm((D, D), BF16), vm((D, D), BF16), vm((D, D), BF16), vm((D, D), BF16),
            vm((D, 3 * D), BF16), vm((D, D), BF16),
            vm((3 * D // 2, D), U32), vm((D // 2, D), U32),
            vm((G, D // 2, 128), U32),
            vm((L, D), F32), vm((L // 2, D), U32), vm((L // 2, D), U32),
            vm((NSEG, L, D), BF16),
            vm((2, G, 128, 128), F32), vm((2, G, 16, 128), F32), vm((H, 128), F32),
            vm((G, L, 128), F32), vm((G, HALO + L, 128), F32), vm((G, HALO + L, 128), F32),
            vm((2, G, HALO, 128), F32), vm((2, G, HALO, 128), F32),
            pltpu.SemaphoreType.DMA((NSEG + 6,)), pltpu.SemaphoreType.DMA((NSEG,)),
        ],
        compiler_params=pltpu.CompilerParams(vmem_limit_bytes=110 * 2 ** 20),
    )(A_x.reshape(S, D), A_wq, A_wk, A_wv, A_wo, A_beta, B_wqkv, B_wo)
    return out.reshape(A_x.shape)
```

```python
import math

import jax
import jax.numpy as jnp
from jax import lax
import jax.experimental.pallas as pl
import jax.experimental.pallas.tpu as pltpu

HV = 4
NIT = 8

S = 2048
D = 1024
H = 32
DH = D // H
NSEG = 4
L = S // NSEG
WIN, DIL = 8, 2
HALO = 16
G = D // 128
NP = G // 2
CH = 128
NCH = L // CH
PITCH = DH // 2 + 1
LOG2E = math.log2(math.e)
QSCALE = DH ** -0.5 * LOG2E
NEG = -1e9
HA, OA, HB, OB = 0, 2, 4, 6

F32, BF16, U32 = jnp.float32, jnp.bfloat16, jnp.uint32
NN = (((1,), (0,)), ((), ()))
NT = (((1,), (1,)), ((), ()))


def _dot(a, b, dims=NN):
    return lax.dot_general(a, b, dims, preferred_element_type=F32)


def _pack(x):
    return pltpu.bitcast(x.astype(BF16), U32)


def _unpack(x):
    return pltpu.bitcast(x, BF16)


def _cat(xs, axis):
    return xs[0] if len(xs) == 1 else jnp.concatenate(xs, axis=axis)


def _tree(fn, xs):
    while len(xs) > 1:
        xs = [fn(xs[i], xs[i + 1]) if i + 1 < len(xs) else xs[i] for i in range(0, len(xs), 2)]
    return xs[0]


def _cols(x):
    return [x[:, g * 128:(g + 1) * 128] for g in range(x.shape[1] // 128)]


def _row_mean(x):
    c = _cols(x)
    lo, hi = [jnp.sum(_tree(jnp.add, part), axis=-1, keepdims=True) for part in (c[:G // 2], c[G // 2:])]
    return (lo + hi) * (1.0 / D)


def _phi(t):
    return jnp.maximum(t, 0.0) + jnp.exp(jnp.minimum(t, 0.0))


def _rcp(x):
    return pltpu.reciprocal(x, approx=False, full_range=False)


def _iota(shape, dim):
    return lax.broadcasted_iota(jnp.int32, shape, dim)


def _halves(x):
    c = _cols(x)
    return _cat(c[0::2], 1), _cat(c[1::2], 1)


def _lhs7(block, put):
    a11 = block(0, 0)
    yield put(2, a11)
    a22 = block(1, 1)
    yield put(3, a22) | put(0, a11 + a22)
    a12 = block(0, 1)
    yield put(4, a11 + a12) | put(6, a12 - a22)
    a21 = block(1, 0)
    yield put(1, a21 + a22) | put(5, a21 - a11)


def _rhs7(b11, b12, b21, b22):
    return [b11 + b22, b11, b12 - b22, b21 - b11, b22, b11 + b12, b21 + b22]


def _strassen(prod, emit):
    m6 = prod(5)
    yield
    m2 = prod(1)
    c22 = m6 - m2
    yield
    m4 = prod(3)
    emit(1, 0, m2 + m4)
    yield
    m1 = prod(0)
    c22 = c22 + m1
    c11 = m4 + m1
    yield
    m3 = prod(2)
    emit(1, 1, c22 + m3)
    yield
    m5 = prod(4)
    emit(0, 1, m3 + m5)
    c11 = c11 - m5
    yield
    emit(0, 0, c11 + prod(6))
    yield


def _chain(*gens):
    for g in gens:
        yield from g


def _idle(n):
    for _ in range(n):
        yield


def _spaced(gen, gap):
    for x in gen:
        yield x
        yield from _idle(gap - 1)


def _drain(gen):
    for _ in gen:
        pass


def _run(order, **gens):
    for ch in order.replace(" ", ""):
        next(gens[ch])
    for name, g in gens.items():
        assert next(g, _run) is _run, name


class _Buf:
    def __init__(self, ref, z):
        self.ref, self.z = ref, z

    def __setitem__(self, idx, val):
        idx = idx if isinstance(idx, tuple) else (idx,)
        self.ref[(0,) + idx] = _pack(val) if self.ref.dtype == U32 else val

    def __getitem__(self, idx):
        idx = idx if isinstance(idx, tuple) else (idx,)
        val = self.ref[(self.z,) + idx]
        return _unpack(val) if self.ref.dtype == U32 else val


def _kernel(x_hbm, wq_hbm, wk_hbm, wv_hbm, wo_hbm, beta_ref, wqkv_hbm, wob_hbm, out_hbm,
            xin, wa_raw, wqkv_raw, wob_raw, wa7, wb7, wob7, tmp, ostage,
            mem, gate, bias, ktail, vtail, sems, osem, scratch, zero):
    def x_copy(i):
        return pltpu.make_async_copy(x_hbm.at[pl.ds(i * 2 * CH, 2 * CH)], xin.at[i], sems.at[i])

    def wa_copy(m, n):
        col = n * 256 if isinstance(n, int) else pl.multiple_of(n * 256, 256)
        return pltpu.make_async_copy((wk_hbm, wq_hbm, wv_hbm, wo_hbm)[m].at[:, pl.ds(col, 256)],
                                     wa_raw.at[m * NP + n], sems.at[2 * NSEG + m * NP + n])

    wb_copies = [pltpu.make_async_copy(wqkv_hbm, wqkv_raw, sems.at[2 * NSEG + 4 * NP]),
                 pltpu.make_async_copy(wob_hbm, wob_raw, sems.at[2 * NSEG + 4 * NP + 1])]
    x_copy(0).start()
    for m in range(3):
        wa_copy(m, 0).start()
    x_copy(1).start()

    b = beta_ref[...].astype(F32).reshape(1, H)
    b = jnp.where(_iota((H, H), 0) == _iota((H, H), 1), jnp.broadcast_to(b, (H, H)), 0.0)
    b = jnp.sum(b, axis=1, keepdims=True)
    gate[...] = jnp.broadcast_to(1.0 / (1.0 + jnp.exp(-b)), (H, 128)).reshape(NP, 8, 128)
    bias[...] = jnp.where(_iota((CH, CH), 0) <= _iota((CH, CH), 1), 0.0, NEG)

    def clear(i, carry):
        zero[i] = 0
        mem[i] = jnp.zeros(mem.shape[1:], F32)
        ktail[i] = jnp.zeros(ktail.shape[1:], F32)
        vtail[i] = jnp.zeros(vtail.shape[1:], F32)
        scratch["ot"][1][0, i] = jnp.zeros((2, 128, CH), F32)
        return carry

    lax.fori_loop(0, 2, clear, 0)
    z = zero[1]
    st = jax.tree.map(lambda r: _Buf(r, z), scratch)
    ops = scratch["ops"]

    def put_operand(slot, b, n):
        def put(i, a):
            a = _pack(a)
            ops[slot][0, i, pl.ds(8 * b, 8), pl.ds(n * 128, 128)] = a
            return a

        return put

    def norm_stats(x, stat):
        for b in range(2 * CH // 16):
            rows = pl.ds(16 * b, 16)
            v = x[rows]
            m = _row_mean(v)
            d = v - m
            stat[0, rows] = jnp.broadcast_to(m, (16, 128))
            stat[1, rows] = jnp.broadcast_to(lax.rsqrt(_row_mean(d * d) + 1e-5), (16, 128))

    def norm_apply(x, stat, slot):
        for b in range(CH // 16):
            for n in range(NP):
                def block(r, s):
                    rows = pl.ds(r * CH + 16 * b, 16)
                    return (x[rows, pl.ds((2 * n + s) * 128, 128)] - stat[0, rows]) * stat[1, rows]

                yield _tree(jnp.bitwise_or, list(_lhs7(block, put_operand(slot, b, n))))

    def prep_a(first, stride, count):
        def body(i, carry):
            u = first + i * stride
            for k in range(D // 32):
                r0 = k // 8 * 2 * CH + k % 8 * 16
                top, bot = [wa_raw[u, pl.ds(r0 + r * CH, 16), :].astype(F32) for r in range(2)]
                for j, w in enumerate(_cols(_pack(_cat(_rhs7(*_cols(top), *_cols(bot)), 1)))):
                    wa7[u, j, pl.ds(8 * k, 8), :] = w
            return carry

        lax.fori_loop(0, count, body, 0)

    def spread_heads(dst, i, w):
        for h in range(H):
            dst[0, i, pl.ds(h * PITCH, DH // 2), :] = w[h * DH // 2:(h + 1) * DH // 2]

    def head_minor(src, i, d, h0):
        w = src[z, i, pl.ds(h0 * PITCH + d // 2, 16, stride=PITCH), :]
        return lax.bitcast_convert_type(w & jnp.uint32(0xFFFF0000) if d % 2 else w << 16, F32)

    def prep_b():
        def gather(src, dst, col, transposed):
            for k in range(D // 32):
                d, h0 = k // 8 * 8 + k % 8 // 2, k % 2 * 16
                (a, b), (c, e) = [[head_minor(src, i, d + 4 * r, h0) for i in range(2)] for r in range(2)]
                ws = _rhs7(a, c, b, e) if transposed else _rhs7(a, b, c, e)
                for j, w in enumerate(_cols(_pack(_cat(ws, 1)))):
                    dst[j, pl.ds(8 * k, 8), pl.ds(col, 128)] = w

        def qkv(i, carry):
            m = i // 2
            for a in range(2):
                for j in range(2):
                    rows = pl.ds(pl.multiple_of((i % 2 * 4 + 2 * a + j) * 128, 128), 128)
                    w = wqkv_raw[rows, pl.ds(pl.multiple_of(m * D, D), D)]
                    spread_heads(tmp[a], j, pltpu.bitcast(w.T, U32))
            for a in range(2):
                gather(tmp[a], wb7.at[m], pl.multiple_of((i % 2 * 2 + a) * 128, 128), True)
            return carry

        def out(n, carry):
            w = pltpu.bitcast(wob_raw[:, pl.ds(pl.multiple_of(n * 256, 256), 256)], U32)
            for j, wj in enumerate(_cols(w)):
                spread_heads(tmp[0], j, wj)
            gather(tmp[0], wob7, pl.multiple_of(n * 128, 128), False)
            return carry

        lax.fori_loop(0, 6, qkv, 0)
        lax.fori_loop(0, NP, out, 0)

    x_copy(0).wait()
    st["xb"][0][...] = xin[0].astype(F32)
    norm_stats(st["xb"][0], st["stat"][0])
    _drain(norm_apply(st["xb"][0], st["stat"][0], HA))
    for m in range(3):
        wa_copy(m, 0).wait()
    for n in (1, 2):
        for m in range(3):
            wa_copy(m, n).start()
    prep_a(0, NP, 3)
    x_copy(1).wait()
    st["xb"][1][...] = xin[1].astype(F32)

    def out_copy(s):
        return pltpu.make_async_copy(ostage.at[s], out_hbm.at[pl.ds(s * L, L)], osem.at[s])

    def project(slot, rhs, emit, fill, dims=NN):
        def prod(i):
            rows = []
            for b in range(CH // 16):
                mark = next(fill, None)
                if mark is not None:
                    ops[slot][0, 7, pl.ds(8 * b, 8), pl.ds(0, 128)] = mark
                rows.append(ops[slot][z, i, pl.ds(8 * b, 8)])
            return _dot(_unpack(_cat(rows, 0)), _unpack(rhs(i)), dims)

        return _strassen(prod, emit)

    def step(it, carry):
        seg, pair = (it // 2) % NSEG, it % 2

        nxt, cur = st["nxt"], st["cur"]

        def a_proj(m, n, c, fill):
            def emit(r, e, y):
                j = 2 * c + r
                if m == 0:
                    pk = _phi(y)
                    nxt["k"][e, j] = y
                    nxt["pk"][e, j] = pk
                    nxt["z"][e, j] = jnp.sum(pk.reshape(CH // 8, 8, 128), axis=0)
                elif m == 1:
                    nxt["qt"][e, j] = (y * QSCALE).astype(BF16).T
                    nxt["pq"][e, j] = _phi(y)
                else:
                    nxt["vt"][e, j] = y.astype(BF16).T

            return project(HA + c, lambda i: wa7[m * NP + n, i], emit, fill)

        def a_scores(src, e):
            blank = jnp.zeros((DH, CH), BF16)
            for j in range(NCH):
                qt = src["qt"][e, j]
                qm = _cat([_cat([qt[a * DH:(a + 1) * DH] if a == hh else blank for a in range(4)], 0)
                           for hh in range(4)], 1)
                sc = _dot(_cat([src["k"][e, i] for i in range(j + 1)], 0), qm)
                blks = [sc[i * CH:(i + 1) * CH] for i in range(j + 1)]
                blks[j] = blks[j] + _cat([bias[...]] * 4, 1)
                for i, blk in enumerate(blks):
                    st["s"][e][j][pl.ds(i * CH, CH)] = blk
                top = jnp.max(_cat(blks, 0), axis=0, keepdims=True)
                st["s"][e][j][pl.ds((j + 1) * CH, 8)] = jnp.broadcast_to(top, (8, 4 * CH))
                yield

        def a_values(src, n, e):
            pq = _cat([src["pq"][e, j] for j in range(NCH)], 0)
            r = _dot(mem[pair, n, e].astype(BF16), pq, NT)
            for j in range(NCH):
                st["r"][e][j] = r[:136, j * CH:(j + 1) * CH]
            yield
            for j in range(NCH):
                acc, l = [None] * 4, [None] * 4
                for h0 in range(0, 4, HV):
                    for i in range(j + 1):
                        for hh in range(h0, h0 + HV):
                            lanes = pl.ds(hh * CH, CH)
                            top = st["s"][e][j][pl.ds((j + 1) * CH, 8), lanes]
                            p = jnp.exp2(st["s"][e][j][pl.ds(i * CH, CH), lanes] - _cat([top] * (CH // 8), 0))
                            for a in reversed(range(CH // 8)):
                                l[hh] = p[8 * a:8 * a + 8] if l[hh] is None else l[hh] + p[8 * a:8 * a + 8]
                            o = _dot(src["vt"][e, i, pl.ds(hh * DH // 2, DH // 2)], p.astype(BF16))
                            acc[hh] = o if acc[hh] is None else acc[hh] + o
                            if i == j:
                                gt = gate[n, pl.ds(4 * e + hh, 1), :]
                                rden = _rcp(st["r"][e][j, pl.ds(128 + hh, 1)] + 1e-6)
                                rl = _rcp(jnp.sum(l[hh], axis=0, keepdims=True))
                                st["ot"][j // 2][j % 2, e, pl.ds(hh * DH, DH)] = (
                                    acc[hh] * ((1.0 - gt) * rl) + st["r"][e][j, pl.ds(hh * DH, DH)] * (gt * rden))
                        yield

        def a_operands(n, c):
            def put(i, a):
                a = pltpu.bitcast(a.astype(BF16).T, U32)
                ops[OA + c][0, i, :, pl.ds(col, 128)] = a
                return a[-8:]

            col = n * 128 if isinstance(n, int) else pl.multiple_of(n * 128, 128)
            return _lhs7(lambda r, e: st["ot"][c][r, e], put)

        def a_update(src, n):
            row, head = _iota((144, 128), 0), _iota((144, 128), 1) // DH
            own = jnp.where(row < 128, row // DH, row - 128) == head
            for e in range(2):
                vt = _cat([src["vt"][e, j] for j in range(NCH)], 1)
                pk = _cat([src["pk"][e, j] for j in range(NCH)], 0)
                zs = jnp.sum(_tree(jnp.add, [src["z"][e, j] for j in range(NCH)]), axis=0, keepdims=True)
                new = _cat([_dot(vt, pk), jnp.broadcast_to(zs, (16, 128))], 0)
                mem[pair, n, e] = mem[pair, n, e] + jnp.where(own, new, 0.0)
                yield

        def a_out(c, fill):
            for n in range(NP):
                def emit(r, s, y):
                    at = (pl.ds(r * CH, CH), pl.ds((2 * n + s) * 128, 128))
                    st["xa"][c][at] = st["xb"][c][at] + y

                yield from project(OA + c, lambda i: wa7[3 * NP + n, i], emit, fill)

        qb, kb, vb = st["qb"], st["kb"], st["vb"]

        def b_proj(c, m, fill):
            for n in range(NP):
                def emit(r, s, y):
                    if m == 0:
                        qb[c][2 * n + s, pl.ds(r * CH, CH)] = y * QSCALE
                    else:
                        (kb, vb)[m - 1][2 * n + s, pl.ds(HALO + (2 * c + r) * CH, CH)] = y

                _drain(project(HB + c, lambda i: wb7[m, i, pl.ds(n * CH // 2, CH // 2), :], emit, fill, NT))

        def b_logits(c):
            for b in range(2 * CH // 16):
                t0 = 2 * c * CH + 16 * b
                q = [qb[c][g, pl.ds(16 * b, 16)] for g in range(G)]
                for w in range(WIN):
                    rows = pl.ds(HALO + t0 - DIL * w, 16)
                    a = q[0] * kb[0, rows]
                    for g in range(1, G):
                        a = a + q[g] * kb[g, rows]
                    a = (a + pltpu.roll(a, 64, 1)) + (pltpu.roll(a, 32, 1) + pltpu.roll(a, 96, 1))
                    if t0 < DIL * w:
                        a = jnp.where(_iota((16, 128), 0) + (seg * L + t0) >= DIL * w, a, NEG)
                    st["lb"][c][w, pl.ds(16 * b, 16)] = a

        def b_probs(c):
            for b in range(2 * CH // 8):
                logits = [st["lb"][c][w, pl.ds(8 * b, 8)] for w in range(WIN)]
                m = _tree(jnp.maximum, logits)
                p = [jnp.exp2(a - m) for a in logits]
                for w in range(WIN):
                    qb[c][w, pl.ds(8 * b, 8)] = p[w]
                l = _tree(jnp.add, p)
                qb[c][WIN, pl.ds(8 * b, 8)] = l
                yield lax.bitcast_convert_type(l, U32)

        def b_values(c):
            for b in range(CH // 16):
                for n in range(NP):
                    def block(r, s):
                        rows = pl.ds(r * CH + 16 * b, 16)
                        t0 = HALO + (2 * c + r) * CH + 16 * b
                        a = qb[c][0, rows] * vb[2 * n + s, pl.ds(t0, 16)]
                        for w in range(1, WIN):
                            a = a + qb[c][w, rows] * vb[2 * n + s, pl.ds(t0 - DIL * w, 16)]
                        return a * _rcp(qb[c][WIN, rows])

                    yield from _lhs7(block, put_operand(OB + c, b, n))

        def b_out(c, fill):
            nseg = jnp.minimum(seg + 1, NSEG - 1)
            for n in range(NP):
                def emit(r, s, y):
                    rows, cols = pl.ds((2 * c + r) * CH, CH), pl.ds((2 * n + s) * 128, 128)
                    x = st["xa"][c][pl.ds(r * CH, CH), cols] + y
                    ostage[seg, rows, cols] = x.astype(BF16)
                    st["xb"][c][pl.ds(r * CH, CH), cols] = jnp.where(
                        pair == 1, xin[2 * nseg + c, pl.ds(r * CH, CH), cols].astype(F32), x)

                _drain(project(OB + c, lambda i: wob7[i, :, pl.ds(n * 128, 128)], emit, fill))

        def norm(x, c, slot, gap):
            norm_stats(st[x][c], st["stat"][c])
            return _chain(_idle(64), _spaced(norm_apply(st[x][c], st["stat"][c], slot + c), gap))

        def done(fill):
            assert next(fill, done) is done

        fill = norm("xb", 1, HA, 3)
        for c in range(2):
            for m in range(3):
                _drain(a_proj(m, 0, c, fill))
            done(fill)
        v = "Pv" * 2 if HV == 2 else "PPv"

        def stage(n, carry):
            @pl.when(it == 0)
            def _():
                for m in range(3):
                    wa_copy(m, n + 1).wait()

                @pl.when(n == 0)
                def _():
                    for c in [wa_copy(m, NP - 1) for m in range(3)] + [wa_copy(3, k) for k in range(NP)] + wb_copies:
                        c.start()
                    for i in range(2, 2 * NSEG):
                        x_copy(i).start()

                prep_a(n + 1, NP, 3)

            for name in sorted(cur):
                cur[name][...] = nxt[name][...]
            fill = _chain(_idle(24), _spaced(a_operands(jnp.maximum(n - 1, 0), 1), 8), _idle(8 * 23), _spaced(a_operands(n, 0), 8))
            grp = "Q v Q" + v * 3 + "Q" + v * 3 + "Q" + v * 4
            _run("PP" + grp + grp + "uu",
                 P=_chain(*[a_proj(m, n + 1, c, fill) for m in range(3) for c in range(2)]),
                 Q=_chain(a_scores(cur, 0), a_scores(cur, 1)), v=_chain(a_values(cur, n, 0), a_values(cur, n, 1)),
                 u=a_update(cur, n))
            done(fill)
            return carry

        lax.fori_loop(0, NP - 1, stage, 0)

        @pl.when(it == 0)
        def _():
            for k in range(NP):
                wa_copy(3, k).wait()
            prep_a(3 * NP, 1, NP)
            for c in wb_copies:
                c.wait()
            prep_b()
            for i in range(2, 2 * NSEG):
                x_copy(i).wait()

        kb[:, pl.ds(0, HALO)] = ktail[pair]
        vb[:, pl.ds(0, HALO)] = vtail[pair]
        k = 4 // HV
        _run("oooo Q v Q R w" + "v" * k + "R" + "vv" * k + "Q" + "w" * k + "R" + "ww" * k + "oooo Q" + "v" * k
             + "R" + "v" * k + v * 5 + v.replace("v", "w") * 7 + "uu PPPP oooo",
             Q=a_scores(nxt, 0), R=a_scores(nxt, 1), v=a_values(nxt, NP - 1, 0), w=a_values(nxt, NP - 1, 1),
             u=a_update(nxt, NP - 1), P=a_out(0, _idle(0)),
             o=_chain(a_operands(NP - 2, 1), a_operands(NP - 1, 0), a_operands(NP - 1, 1)))
        fill = norm("xa", 0, HB, 4)
        _drain(a_out(1, fill))
        done(fill)
        fill = norm("xa", 1, HB, 8)
        for c in range(2):
            b_proj(c, 0, fill)
            b_proj(c, 1, fill)
            done(fill)
            b_logits(c)
            fill = _chain(_idle(156), _spaced(b_probs(c), 2))
            b_proj(c, 2, fill)
            done(fill)
            fill = _chain(_idle(12), _spaced(b_values(c), 3 - 2 * c))
        b_out(0, fill)
        done(fill)
        fill = norm("xb", 0, HA, 4)
        b_out(1, fill)
        done(fill)
        ktail[pair] = kb[:, pl.ds(L, HALO)]
        vtail[pair] = vb[:, pl.ds(L, HALO)]

        @pl.when((pair == 1) & (it >= NIT - 8))
        def _():
            out_copy(seg).start()

        return carry

    lax.fori_loop(0, NIT, step, 0)
    for s in range(NSEG):
        out_copy(s).wait()


@jax.jit
def pallas_interleave_layers__memory_aug_infini_attn__sliding_local_dilated__prompt_kernel(
    A_x, A_wq, A_wk, A_wv, A_wo, A_beta, B_x, B_wqkv, B_wo,
):
    del B_x
    hbm = pl.BlockSpec(memory_space=pl.ANY)
    vm = pltpu.VMEM
    out = pl.pallas_call(
        _kernel,
        name="infini_dilated",
        out_shape=jax.ShapeDtypeStruct((S, D), BF16),
        in_specs=[hbm, hbm, hbm, hbm, hbm, pl.BlockSpec(memory_space=pltpu.VMEM), hbm, hbm],
        out_specs=hbm,
        scratch_shapes=[
            vm((2 * NSEG, 2 * CH, D), BF16),
            vm((4 * NP, D, 256), BF16), vm((D, 3 * D), BF16), vm((D, D), BF16),
            vm((4 * NP, 7, D // 4, 128), U32), vm((3, 7, D // 4, D // 2), U32), vm((7, D // 4, D // 2), U32),
            [vm((1, 2, H * PITCH, 128), U32)] * 2,
            vm((NSEG, L, D), BF16),
            vm((2, NP, 2, 144, 128), F32), vm((NP, 8, 128), F32), vm((CH, CH), F32),
            vm((2, G, HALO, 128), F32), vm((2, G, HALO, 128), F32),
            pltpu.SemaphoreType.DMA((2 * NSEG + 4 * NP + 2,)), pltpu.SemaphoreType.DMA((NSEG,)),
            dict(
                **{k: dict(z=vm((1, 2, NCH, 8, 128), F32),
                           **{a: vm((1, 2, NCH, CH // 2, 128), U32) for a in ("k", "pk", "qt", "pq", "vt")})
                   for k in ("nxt", "cur")},
                ops=[vm((1, 8, CH // 2, D // 2), U32)] * 8,
                **{k: [vm((1, 2 * CH, D), F32)] * 2 for k in ("xa", "xb")},
                **{k: vm((1, G, HALO + L + 24, 128), F32) for k in ("kb", "vb")},
                **{k: [vm((1, G + 4, 2 * CH + 8, 128), F32)] * 2 for k in ("qb", "lb")},
                s=[[vm((1, (j + 1) * CH + 8, 4 * CH), F32) for j in range(NCH)]] * 2,
                r=[vm((1, NCH, 136, CH), F32)] * 2,
                ot=[vm((1, 2, 2, 128, CH), F32)] * 2,
                stat=[vm((1, 2, 2 * CH, 128), F32)] * 2,
            ),
            pltpu.SMEM((2,), jnp.int32),
        ],
        compiler_params=pltpu.CompilerParams(vmem_limit_bytes=110 * 2 ** 20),
    )(A_x.reshape(S, D), A_wq, A_wk, A_wv, A_wo, A_beta, B_wqkv, B_wo)
    return out.reshape(A_x.shape)
```

```python
import math

import jax
import jax.numpy as jnp
from jax import lax
import jax.experimental.pallas as pl
import jax.experimental.pallas.tpu as pltpu

S = 2048
D = 1024
H = 32
DH = D // H
NSEG = 4
L = S // NSEG
WIN, DIL = 8, 2
HALO = 16
G = D // 128
NP = G // 2
CH = 128
NCH = L // CH
PITCH = DH // 2 + 1
QSCALE = DH ** -0.5 * math.log2(math.e)
NEG = -1e9
HA, OA, HB, OB = 0, 2, 4, 6
SEM_BETA, SEM_WB, SEM_PANEL, SEM_OUT = 3, 5, 8, 16

STAGE_ORDER = ("uuPPQQPPPvPPvQPvPvPvPQPvPvvPPvvPPvQQPPvPvvPvPvPPvPPPvQPPvvPvQPvPvPPvPvPPvPvPvPvvPvPvrr")
LAST_ORDER = ("ooooQQRvvRQwvwvRwwooooQvRPvPvvPvPvPPvvPPvPvPPvwPPvPPwwPwPwPPwPPwPwwPPwPwwuuPPPoooo")
ANC = 17
NRM = 16
PART = ("HSR")

F32, BF16, I32 = jnp.float32, jnp.bfloat16, jnp.int32
NN = (((1,), (0,)), ((), ()))
NT = (((1,), (1,)), ((), ()))


def _dot(a, b, dims=NN):
    return lax.dot_general(a, b, dims, preferred_element_type=F32)


def _pack(x):
    return pltpu.bitcast(x.astype(BF16), I32)


def _unpack(x):
    return pltpu.bitcast(x, BF16)


def _cat(xs, axis):
    return xs[0] if len(xs) == 1 else lax.concatenate(xs, axis)


def _tree(fn, xs):
    while len(xs) > 1:
        xs = [fn(xs[i], xs[i + 1]) if i + 1 < len(xs) else xs[i] for i in range(0, len(xs), 2)]
    return xs[0]


def _cols(x):
    return [x[:, g * 128:(g + 1) * 128] for g in range(x.shape[1] // 128)]


def _fold(fn, x):
    return fn(x.reshape(x.shape[0] // 8, 8, x.shape[1]), axis=0)


def _digest(x, rows=8):
    for n in (4 * rows, 2 * rows, rows):
        x = x[:n] | x[-n:]
    return x


def _iota(shape, dim):
    return lax.broadcasted_iota(I32, shape, dim)


def _row_mean(x):
    c = _cols(x)
    return _tree(lax.add, [jnp.sum(c[i] + c[i + 4], axis=-1, keepdims=True) for i in range(4)]) * (1.0 / D)


def _phi(t):
    return jnp.maximum(t, 0.0) + jnp.exp(jnp.minimum(t, 0.0))


def _rcp(x):
    return pltpu.reciprocal(x, approx=False, full_range=False)


def _rotate_quarters(xs, sign):
    for bit in (1, 2):
        on = _iota(xs[0].shape, 1) & (DH * bit) != 0
        xs = [lax.select(on, xs[(i + sign * bit) % 4], xs[i]) for i in range(4)]
    return xs


def _rotate_rows(x, sign):
    n = x.shape[0] // 4
    return _cat(_rotate_quarters([x[i * n:(i + 1) * n] for i in range(4)], sign), 0)


def _exchange(xs):
    ys = _rotate_quarters(xs, 1)
    return [ys[-i % 4] for i in range(4)]


def _lhs7(block, put):
    a11 = block(0, 0)
    yield put((2, a11))
    a22 = block(1, 1)
    yield put((3, a22), (0, a11 + a22))
    a12 = block(0, 1)
    yield put((4, a11 + a12), (6, a12 - a22))
    a21 = block(1, 0)
    yield put((1, a21 + a22), (5, a21 - a11))


def _rhs7(b11, b12, b21, b22):
    return [b11 + b22, b11, b12 - b22, b21 - b11, b22, b11 + b12, b21 + b22]


def _strassen(prod, emit, park):
    m6 = prod(5)
    yield
    m2 = prod(1)
    park[0][...] = m6 - m2
    yield
    m4 = prod(3)
    emit(1, 0, m2 + m4)
    yield
    m1 = prod(0)
    c22 = park[0][...] + m1
    park[1][...] = m4 + m1
    yield
    m3 = prod(2)
    emit(1, 1, c22 + m3)
    yield
    m5 = prod(4)
    emit(0, 1, m3 + m5)
    c11 = park[1][...] - m5
    yield
    emit(0, 0, c11 + prod(6))
    yield


def _chain(*gens):
    for g in gens:
        yield from g


def _idle(n):
    for _ in range(n):
        yield


def _spaced(gen, *gaps):
    for i, x in enumerate(gen):
        yield x
        yield from _idle(gaps[i % len(gaps)] - 1)


def _merge(a, b):
    while True:
        xs = [x for x in (next(a, _merge), next(b, _merge)) if x is not _merge]
        if not xs:
            return
        xs = [x for x in xs if x is not None]
        yield _tree(lax.bitwise_or, xs) if xs else None


def _drain(gen):
    for _ in gen:
        pass


def _run(order, **gens):
    for ch in order.replace(" ", ""):
        next(gens[ch])
    for name, g in gens.items():
        assert next(g, _run) is _run, name


class _Buf:
    def __init__(self, ref, z):
        self.ref, self.z = ref, z

    def __setitem__(self, idx, val):
        self.ref[(0,) + (idx if isinstance(idx, tuple) else (idx,))] = val

    def __getitem__(self, idx):
        return self.ref[(self.z,) + (idx if isinstance(idx, tuple) else (idx,))]


def _kernel(x_hbm, wq_hbm, wk_hbm, wv_hbm, wo_hbm, beta_hbm, wqkv_hbm, wob_hbm, out_hbm,
            xin, xout, wa_raw, wqkv_raw, wob_raw, wa7, mem, gate, bias, ktail, vtail, scratch, zero, sems, beta):
    def panel_copy(m, n):
        src, col = ((wk_hbm, wq_hbm, wv_hbm)[m], n) if n < NP else (wo_hbm, 3 * (n - NP) + m)
        return pltpu.make_async_copy(src.at[:, pl.ds(col * 256, 256)], wa_raw.at[n, m],
                                     sems.at[SEM_PANEL + (2 + n if n else m)])

    def x_copy(i, n=1):
        return pltpu.make_async_copy(x_hbm.at[pl.ds(i, n)], xin.at[pl.ds(i, n)], sems.at[i])

    def wb_copy(m):
        col = m * D if isinstance(m, int) else pl.multiple_of(m * D, D)
        return pltpu.make_async_copy(wqkv_hbm.at[:, pl.ds(col, D)], wqkv_raw.at[m], sems.at[SEM_WB + m])

    def out_copy(*at):
        return pltpu.make_async_copy(xout.at[at], out_hbm.at[at], sems.at[SEM_OUT])

    beta_copy = pltpu.make_async_copy(beta_hbm, beta, sems.at[SEM_BETA])
    beta_copy.start()
    x_copy(0).start()
    for n in range(NP + 1):
        if n >= 2:
            wb_copy(n - 2).start()
        for m in range(3):
            panel_copy(m, n).start()
            if (m, n) == (1, 0):
                x_copy(1).start()
    last_copies = [panel_copy(0, NP + 1), pltpu.make_async_copy(wob_hbm, wob_raw, sems.at[SEM_OUT + 1]),
                   x_copy(2, 2)]
    for c in last_copies:
        c.start()
    x_copy(4, 4).start()

    def clear(i, carry):
        zero[i] = 0
        mem[i] = jnp.zeros(mem.shape[1:], F32)
        ktail[i] = jnp.zeros(ktail.shape[1:], F32)
        vtail[i] = jnp.zeros(vtail.shape[1:], F32)
        scratch["ot"][1][0, i] = jnp.zeros((2, 128, CH), F32)
        return carry

    lax.fori_loop(0, 2, clear, 0)
    z = zero[1]
    st = jax.tree.map(lambda r: _Buf(r, z), scratch)
    ops, wb7, tmp, nxt, cur, qb, kb, vb = [st[k] for k in ("ops", "wb7", "tmp", "nxt", "cur", "qb", "kb", "vb")]

    def prep_panel(m, n):
        for k in range(NP):
            rows = [pl.ds((2 * k + r) * CH, CH) for r in range(2)]
            ws = _rhs7(*[w for r in rows for w in _cols(wa_raw[n, m, r, :].astype(F32))])
            out = _cols(_pack(_cat([ws[j] for j in (0, 2, 3, 5, 6)], 1)))
            out += [_pack(wa_raw[n + z, m, rows[r], pl.ds(r * 128, 128)]) for r in range(2)]
            for j, w in zip((0, 2, 3, 5, 6, 1, 4), out):
                wa7[n, m, j, pl.ds(k * CH // 2, CH // 2), :] = w
            yield

    def prep_panels(n):
        pltpu.make_async_copy(wa_raw.at[n], wa_raw.at[n], sems.at[SEM_PANEL + 2 + n]).wait()
        lax.fori_loop(0, 3, lambda m, carry: _drain(prep_panel(m, n)), None)

    def spread(m, j, g, w):
        w = _pack(w)
        for h in range(8):
            tmp[m, j, pl.ds((8 * g + h) * PITCH, DH // 2)] = w[h * DH // 2:(h + 1) * DH // 2]
        return w[-8:]

    def spread_qkv(m):
        for j in range(G):
            for g in range(NP):
                yield spread(m, j, g, wqkv_raw[m, pl.ds(j * 128, 128), pl.ds(g * 256, 256)].T)

    def gather(m):
        for k in range(2 * NP):
            ws = [_cat([tmp[m, j, pl.ds(k // 2 * 4 + k % 2 + 2 * r, H, stride=PITCH)] for j in range(s, G, 2)], 1)
                  for r in range(2) for s in range(2)]
            a, b, c, d = [lax.bitcast_convert_type(_cat([w << 16, w & -65536], 0), F32) for w in ws]
            ws = _pack(_cat(_rhs7(a, c, b, d) if m < 3 else _rhs7(a, b, c, d), 0))
            wb7[m][:, pl.ds(k * H, H)] = ws.reshape(7, H, D // 2)
            bits = _cols(_digest(ws, H))
            for half in (bits[0] | bits[1], bits[2] | bits[3]):
                for row in (0, 16, 8, 24):
                    yield half[row:row + 8]

    recent, pending = [], []

    def streamed(y, slots=None):
        recent.extend((y, 16 * b) for b in range(slots or y.shape[0] // 16))

    def result(age):
        y, row = recent[-age]
        return y[row:row + 8, :128]

    def project(slot, rhs, emit, fill, dims=NN):
        def prod(i):
            rows, start = [], 0
            for b in range(CH // 16):
                mark = next(fill, None)
                while b == 0 and pending and pending[0][0] <= len(recent):
                    late = pending.pop(0)[1]
                    mark = late if mark is None else mark | late
                if mark is None:
                    continue
                if len(recent) >= 12 - b:
                    mark = mark | lax.bitcast_convert_type(result(12 - b), I32)
                if b > start:
                    rows.append(ops[slot][i, pl.ds(8 * start, 8 * (b - start))])
                    start = b
                ops[slot][7, pl.ds(8 * b, 8), pl.ds(0, 128)] = mark
            rows.append(ops[slot][i, pl.ds(8 * start, CH // 2 - 8 * start)])
            y = _dot(_unpack(_cat(rows, 0)), _unpack(rhs(i)), dims)
            streamed(y)
            return y

        return _strassen(prod, emit, st["park"])

    def done(fill):
        assert next(fill, done) is done
        recent.clear()
        pending.clear()

    def put_operand(slot, b, n):
        def put(*items):
            packed = _cols(_pack(_cat([a for _, a in items], 1)))
            for (i, _), a in zip(items, packed):
                ops[slot][i, pl.ds(8 * b, 8), pl.ds(n * 128, 128)] = a
            return _tree(lax.bitwise_or, packed)

        return put

    def put_chunk(slot, h):
        h, parts = _cols(h), []
        _drain(_lhs7(lambda r, s: _cat(h[s::2], 1)[r * CH:(r + 1) * CH], lambda *items: parts.extend(items)))
        packed = _pack(_cat([a for _, a in sorted(parts, key=lambda item: item[0])], 0))
        ops[slot][pl.ds(0, 7)] = packed.reshape(7, CH // 2, D // 2)
        return packed

    def norm(x, c, slot, gap):
        x, stat = st[x][c], st["stat"][c]
        for b in range(2 * CH // NRM):
            rows = pl.ds(NRM * b, NRM)
            v = x[rows]
            m = _row_mean(v)
            d = v - m
            stat[0, rows] = jnp.broadcast_to(m, (NRM, 128))
            stat[1, rows] = jnp.broadcast_to(lax.rsqrt(_row_mean(d * d) + 1e-5), (NRM, 128))

        def apply():
            h = (x[...] - _cat([stat[0]] * G, 1)) * _cat([stat[1]] * G, 1)
            bits = _cols(_digest(put_chunk(slot + c, h), CH // 2))
            bits = [bits[0] | bits[1], bits[2] | bits[3]]
            for b in range(CH // 16):
                for half in bits:
                    yield half[8 * b:8 * b + 8]

        return _chain(_idle(72), _spaced(apply(), 2 * gap))

    bias[...] = jnp.where(_iota((DH, CH), 0) > _iota((DH, CH), 1) % DH, NEG, 0.0)
    beta_copy.wait()
    b = jnp.broadcast_to(beta[...].astype(F32).reshape(1, H), (H, H))
    b = jnp.sum(jnp.where(_iota((H, H), 0) == _iota((H, H), 1), b, 0.0), axis=1, keepdims=True)
    gate[...] = jnp.broadcast_to(1.0 / (1.0 + jnp.exp(-b)), (H, 128)).reshape(NP, 8, 128)
    x_copy(0).wait()
    x = xin[0].astype(F32)
    st["xb"][0][...] = x
    d = x - jnp.mean(x, axis=-1, keepdims=True)
    put_chunk(HA, d * lax.rsqrt(jnp.mean(d * d, axis=-1, keepdims=True) + 1e-5))
    for m in range(3):
        panel_copy(m, 0).wait()
        _drain(prep_panel(m, 0))
        if m == 1:
            x_copy(1).wait()
            st["xb"][1][...] = xin[1].astype(F32)

    def step(it, carry):
        seg, pair = it // 2, it % 2

        def a_proj(m, n, c, fill):
            def emit(r, e, y):
                j = 2 * c + r
                if m == 0:
                    pk = _phi(y)
                    nxt["k"][e, j], nxt["pk"][e, j] = _cols(_pack(_cat([y, pk], 1)))
                    nxt["z"][e, j] = _fold(jnp.sum, pk)
                    return
                if m == 1:
                    y = _rotate_rows(y, -1)
                    nxt["pq"][e, j] = _pack(_phi(y))
                    y = y * QSCALE
                y = _pack(y.astype(BF16).T)
                nxt["qt" if m == 1 else "vt"][e, j] = y
                pending.append((len(recent) + 40, y[-8:]))

            return project(HA + c, lambda i: wa7[n, m, i], emit, fill)

        def a_recall(n):
            for e in range(2):
                r = _dot(mem[pair, n, e].astype(BF16), _unpack(nxt["pq"][e].reshape(L // 2, 128)), NT)
                st["r"][e][...] = r[:136]
                yield

        def a_update(n):
            row, head = _iota((144, 128), 0), _iota((144, 128), 1) // DH
            own = jnp.where(row < 128, row // DH, row - 128) == head
            for e in range(2):
                vt = _unpack(_cat([nxt["vt"][e, j] for j in range(NCH)], 1))
                zs = jnp.sum(jnp.sum(nxt["z"][e], axis=0), axis=0, keepdims=True)
                new = _cat([_dot(vt, _unpack(nxt["pk"][e].reshape(L // 2, 128))), jnp.broadcast_to(zs, (16, 128))], 0)
                mem[pair, n, e] = mem[pair, n, e] + jnp.where(own, new, 0.0)
                yield

        def a_scores(src, e):
            blank = jnp.zeros((DH // 2, CH), I32)
            quarter = (_iota((CH // 2, CH), 1) // DH - _iota((CH // 2, CH), 0) // (DH // 2)) & 3
            for j in range(NCH):
                qt = src["qt"][e, j]
                top = [None] * 4
                for t in reversed(range(4)):
                    sc = _dot(_unpack(src["k"][e, j, pl.ds(0, (t + 1) * DH // 2)]),
                              _unpack(jnp.where(quarter == t, qt, 0)))
                    sc = _cat([sc[:t * DH]] * (t > 0) + [sc[t * DH:] + bias[...]], 0)
                    st["s"][e][j][pl.ds(j * CH, (t + 1) * DH), pl.ds(t * CH, CH)] = sc
                    top[t] = _fold(jnp.max, sc)
                    if t == 3:
                        streamed(sc, 5)
                top = _cat(_exchange(top), 1)
                if j > 0:
                    heads = [_cat([qt[a * DH // 2:(a + 1) * DH // 2] if a == hh else blank for a in range(4)], 0)
                             for hh in range(4)]
                    sc = _dot(_unpack(src["k"][e, pl.ds(0, j)].reshape(j * CH // 2, 128)), _unpack(_cat(heads, 1)))
                    st["s"][e][j][pl.ds(0, j * CH)] = sc
                    top = jnp.maximum(top, _fold(jnp.max, sc))
                    streamed(sc)
                st["top"][e][j][pl.ds(0, 8)] = jnp.broadcast_to(jnp.max(top, axis=0, keepdims=True), (8, 4 * CH))
                yield

        def a_values(src, n, e):
            def tops(j):
                if len(recent) >= ANC:
                    st["top"][e][j][pl.ds(8, 8), pl.ds(0, 128)] = result(ANC)
                return _cols(st["top"][e][j][pl.ds(0, 8)])

            def probs(j, row, rows, col, top, l):
                p = jnp.exp2(st["s"][e][j][pl.ds(row, rows), pl.ds(col * CH, CH)] - _cat([top] * (rows // 8), 0))
                for a in reversed(range(rows // 16)):
                    l = p[16 * a:16 * a + 16] if l is None else l + p[16 * a:16 * a + 16]
                return p, _fold(jnp.sum, l)

            def mix(i, hh, p):
                return _dot(_unpack(src["vt"][e, i, pl.ds(hh * DH // 2, DH // 2)]), p.astype(BF16))

            def finish(j, hh, acc, l):
                g = gate[n, pl.ds(4 * e + hh, 1), :]
                rden = _rcp(st["r"][e][pl.ds(128 + hh, 1), pl.ds(j * CH, CH)] + 1e-6)
                rl = _rcp(jnp.sum(l, axis=0, keepdims=True))
                st["ot"][j // 2][j % 2, e, pl.ds(hh * DH, DH)] = (
                    acc * ((1.0 - g) * rl) + st["r"][e][pl.ds(hh * DH, DH), pl.ds(j * CH, CH)] * (g * rden))

            for j in range(NCH):
                p, l = zip(*[probs(j, j * CH, (t + 1) * DH, t, top, None)
                             for t, top in enumerate(_exchange(tops(j)))])
                l = _exchange(l)
                p = [_exchange([jnp.zeros((DH // 2, CH), I32)] * a
                               + _cols(_pack(_cat([p[t][a * DH:(a + 1) * DH] for t in range(a, 4)], 1))))
                     for a in range(4)]
                acc = [mix(j, hh, _unpack(_cat([p[a][hh] for a in range(4)], 0))) for hh in range(4)]
                if j == 0:
                    for hh in range(4):
                        finish(j, hh, acc[hh], l[hh])
                yield
                for hp in range(2):
                    for i in range(j):
                        top = tops(j)
                        for hh in (2 * hp, 2 * hp + 1):
                            p, more = probs(j, i * CH, CH, hh, top[hh], None)
                            acc[hh], l[hh] = acc[hh] + mix(i, hh, p), l[hh] + more
                            if i == j - 1:
                                finish(j, hh, acc[hh], l[hh])
                        yield

        def a_operands(n, c):
            col = n * 128 if isinstance(n, int) else pl.multiple_of(n * 128, 128)

            def put(*items):
                out = [_rotate_rows(_pack(a.astype(BF16).T), 1) for _, a in items]
                for (i, _), a in zip(items, out):
                    ops[OA + c][i, :, pl.ds(col, 128)] = a
                return _tree(lax.bitwise_or, [a[-8:] for a in out])

            return _lhs7(lambda r, e: st["ot"][c][r, e], put)

        def a_out(c, fill):
            for n in range(NP):
                def emit(r, s, y):
                    at = (pl.ds(r * CH, CH), pl.ds((2 * n + s) * 128, 128))
                    st["xa"][c][at] = st["xb"][c][at] + y

                yield from project(OA + c, lambda i: wa7[NP + n // 3, n % 3, i], emit, fill)

        def b_proj(c, m, fill):
            for n in range(NP):
                def emit(r, s, y):
                    if m == 0:
                        qb[c][2 * n + s, pl.ds(r * CH, CH)] = y * QSCALE
                    else:
                        (kb, vb)[m - 1][2 * n + s, pl.ds(HALO + (2 * c + r) * CH, CH)] = y

                _drain(project(HB + c, lambda i: wb7[m][i, pl.ds(n * CH // 2, CH // 2)], emit, fill, NT))

        def b_logits(c):
            for b in range(2 * CH // 16):
                t0 = 2 * c * CH + 16 * b
                q = qb[c][pl.ds(0, G), pl.ds(16 * b, 16)]
                for w in range(WIN):
                    a = jnp.sum(q * kb[:, pl.ds(HALO + t0 - DIL * w, 16)], axis=0)
                    a = (a + pltpu.roll(a, 64, 1)) + (pltpu.roll(a, 32, 1) + pltpu.roll(a, 96, 1))
                    if t0 < DIL * w:
                        a = jnp.where(_iota((16, 128), 0) + (seg * L + t0) >= DIL * w, a, NEG)
                    st["lb"][c][w, pl.ds(16 * b, 16)] = a

        def b_probs(c):
            a = st["lb"][c][:, pl.ds(0, 2 * CH)]
            p = jnp.exp2(a - jnp.max(a, axis=0, keepdims=True))
            qb[c][pl.ds(0, WIN), pl.ds(0, 2 * CH)] = p
            l = jnp.sum(p, axis=0)
            st["stat"][c][0] = _rcp(l)
            l = lax.bitcast_convert_type(l, I32)
            for b in range(2 * CH // 8):
                yield l[8 * b:8 * b + 8]

        def b_values(c):
            for b in range(CH // 16):
                for n in range(NP):
                    if len(recent) >= 16:
                        qb[c][WIN, pl.ds(0, 8)] = result(16)
                    o = []
                    for r in range(2):
                        rows = pl.ds(r * CH + 16 * b, 16)
                        t0 = HALO + (2 * c + r) * CH + 16 * b
                        v = _cat([vb[pl.ds(2 * n, 2), pl.ds(t0 - DIL * w, 16)] for w in range(WIN)], 1)
                        a = v.reshape(2, WIN, 16, 128) * qb[c][pl.ds(0, WIN), rows]
                        o.append(jnp.sum(a, axis=1) * st["stat"][c][0, rows])
                    yield from _lhs7(lambda r, s: o[r][s], put_operand(OB + c, b, n))

        def b_out(c, fill):
            following = 2 * jnp.minimum(seg + 1, NSEG - 1) + c
            for n in range(NP):
                def emit(r, s, y):
                    at = (pl.ds(r * CH, CH), pl.ds((2 * n + s) * 128, 128))
                    x = st["xa"][c][at] + y
                    xout[(2 * seg + c,) + at] = x.astype(BF16)
                    st["xb"][c][at] = jnp.where(pair == 1, xin[(following,) + at].astype(F32), x)

                for i, _ in enumerate(project(OB + c, lambda i: wb7[3][i, :, pl.ds(n * 128, 128)], emit, fill)):
                    if (c, n, i) == (1, 2, 1):
                        @pl.when(pair == 1)
                        def _():
                            out_copy(2 * seg).start()
                            out_copy(2 * seg + 1, slice(None), pl.ds(0, D // 2)).start()

        if "H" in PART:
            fill = norm("xb", 1, HA, 3)
            for c in range(2):
                for m in (2, 1, 0):
                    _drain(a_proj(m, 0, c, fill))
                done(fill)
            _drain(a_recall(0))

        def stage(n, carry):
            @pl.when(it == 0)
            def _():
                prep_panels(n + 1)
                wb_copy(n).wait()

            def keep(name):
                for e in range(2):
                    for j in range(NCH):
                        w = nxt[name][e, j]
                        cur[name][e, j] = w
                        yield _digest(w)

            fill = _chain(keep("k"), keep("qt"), keep("vt"), _idle(8),
                          _spaced(a_operands(jnp.maximum(n - 1, 0), 1), 8), _spaced(spread_qkv(n), 6),
                          _spaced(a_operands(n, 0), 8))
            _run(STAGE_ORDER, P=_chain(*[a_proj(m, n + 1, c, fill) for m in (2, 1, 0) for c in range(2)]),
                 Q=_chain(a_scores(cur, 0), a_scores(cur, 1)), v=_chain(a_values(cur, n, 0), a_values(cur, n, 1)),
                 u=a_update(n), r=a_recall(n + 1))
            done(fill)
            return carry

        if "S" in PART:
            lax.fori_loop(0, NP - 1, stage, 0)
        if "R" not in PART:
            xout[0, :16, :128] = _unpack(tmp[0, 0, :8] | ops[OA][0, :8, :128] | ops[OA + 1][0, :8, :128])
            return carry

        @pl.when(it == 0)
        def _():
            prep_panels(NP)
            for c in last_copies:
                c.wait()
            for g, _ in enumerate(prep_panel(0, NP + 1)):
                for j in range(G):
                    spread(3, j, g, wob_raw[pl.ds(g * 256, 256), pl.ds(j * 128, 128)])

        pl.when(it == 1)(x_copy(4, 4).wait)
        kb[:, pl.ds(0, HALO)] = ktail[pair]
        vb[:, pl.ds(0, HALO)] = vtail[pair]
        gather_q = gather(0)
        _run(LAST_ORDER, Q=a_scores(nxt, 0), R=a_scores(nxt, 1), v=a_values(nxt, NP - 1, 0),
             w=a_values(nxt, NP - 1, 1), u=a_update(NP - 1),
             P=a_out(0, _spaced((x for _, x in zip(range(24), gather_q)), 8)),
             o=_chain(a_operands(NP - 2, 1), a_operands(NP - 1, 0), a_operands(NP - 1, 1)))
        fill = _merge(norm("xa", 0, HB, 4), _chain(_idle(60), _spaced(gather_q, 3, 5)))
        _drain(a_out(1, fill))
        done(fill)
        if "T" in PART:
            xout[0, :16, :128] = _unpack(wb7[0][0, :8, :128] | ops[HB][0, :8, :128] | _pack(st["xa"][1][:16, :128]))
            return carry
        for c in range(2):
            if c == 0:
                fill = _chain(_idle(58), _spaced(gather(1), 2, 3), _idle(6),
                              _merge(norm("xa", 1, HB, 4), _spaced(gather(2), 3, 3, 4)))
            else:
                fill = _chain(_idle(12), _spaced(b_values(0), 1, 2, 2), _spaced(gather(3), 3, 3, 4))
            b_proj(c, 0, fill)
            b_proj(c, 1, fill)
            done(fill)
            b_logits(c)
            fill = _chain(_idle(156), _spaced(b_probs(c), 2))
            b_proj(c, 2, fill)
            done(fill)
        fill = _chain(_idle(12), _spaced(b_values(1), 2, 1, 2, 2, 1))
        b_out(0, fill)
        done(fill)
        fill = norm("xb", 0, HA, 4)
        b_out(1, fill)
        done(fill)
        ktail[pair] = kb[:, pl.ds(L, HALO)]
        vtail[pair] = vb[:, pl.ds(L, HALO)]
        pl.when(pair == 1)(out_copy(2 * seg + 1, slice(None), pl.ds(D // 2, D // 2)).start)
        return carry

    lax.fori_loop(0, 2 * NSEG, step, 0)
    pltpu.make_async_copy(xout, out_hbm, sems.at[SEM_OUT]).wait()


@jax.jit
def pallas_interleave_layers__memory_aug_infini_attn__sliding_local_dilated__prompt_kernel(
    A_x, A_wq, A_wk, A_wv, A_wo, A_beta, B_x, B_wqkv, B_wo,
):
    del B_x
    hbm = pl.BlockSpec(memory_space=pl.ANY)
    vm = pltpu.VMEM
    chunks = (2 * NSEG, 2 * CH, D)
    heads = vm((1, 2, NCH, CH // 2, 128), I32)
    scratch = dict(
        ops=[vm((1, 8, CH // 2, D // 2), I32)] * 8,
        wb7=[vm((1, 7, D // 4, D // 2), I32)] * 4,
        tmp=vm((1, 4, G, H * PITCH, 128), I32),
        park=[vm((1, CH, 128), F32)] * 2,
        stat=[vm((1, 2, 2 * CH, 128), F32)] * 2,
        xa=[vm((1, 2 * CH, D), F32)] * 2,
        xb=[vm((1, 2 * CH, D), F32)] * 2,
        nxt=dict(k=heads, qt=heads, vt=heads, pk=heads, pq=heads, z=vm((1, 2, NCH, 8, 128), F32)),
        cur=dict(k=heads, qt=heads, vt=heads),
        s=[[vm((1, (j + 1) * CH, 4 * CH), F32) for j in range(NCH)]] * 2,
        top=[[vm((1, 16, 4 * CH), F32)] * NCH] * 2,
        r=[vm((1, 136, L), F32)] * 2,
        ot=[vm((1, 2, 2, 128, CH), F32)] * 2,
        qb=[vm((1, G + 4, 2 * CH + 8, 128), F32)] * 2,
        lb=[vm((1, WIN, 2 * CH + 8, 128), F32)] * 2,
        kb=vm((1, G, HALO + L + 24, 128), F32),
        vb=vm((1, G, HALO + L + 24, 128), F32),
    )
    out = pl.pallas_call(
        _kernel,
        name="infini_dilated",
        out_shape=jax.ShapeDtypeStruct(chunks, BF16),
        in_specs=[hbm] * 8,
        out_specs=hbm,
        scratch_shapes=[
            vm(chunks, BF16), vm(chunks, BF16),
            vm((NP + 2, 3, D, 256), BF16), vm((3, D, D), BF16), vm((D, D), BF16),
            vm((NP + 2, 3, 7, D // 4, 128), I32),
            vm((2, NP, 2, 144, 128), F32), vm((NP, 8, 128), F32), vm((DH, CH), F32),
            vm((2, G, HALO, 128), F32), vm((2, G, HALO, 128), F32),
            scratch, pltpu.SMEM((2,), I32), pltpu.SemaphoreType.DMA((SEM_OUT + 2,)), vm((H,), BF16),
        ],
        compiler_params=pltpu.CompilerParams(vmem_limit_bytes=110 * 2 ** 20),
    )(A_x.reshape(chunks), A_wq, A_wk, A_wv, A_wo, A_beta, B_wqkv, B_wo)
    return out.reshape(A_x.shape)
```

```python
import math

import jax
import jax.numpy as jnp
from jax import lax
import jax.experimental.pallas as pl
import jax.experimental.pallas.tpu as pltpu

S = 2048
D = 1024
H = 32
DH = D // H
NSEG = 4
L = S // NSEG
WIN, DIL = 8, 2
HALO = 16
G = D // 128
NP = G // 2
CH = 128
NCH = L // CH
PITCH = DH // 2 + 1
QSCALE = DH ** -0.5 * math.log2(math.e)
NEG = -1e9
HA, OA, HB, OB = 0, 2, 4, 6
SEM_BETA, SEM_WB, SEM_PANEL, SEM_OUT = 3, 5, 8, 16

STAGE_ORDER = ("uuPPQQPPPvPPvQPvPvPvPQPvPvvPPvvPPvQQPPvPvvPvPvPPvPPPvQPPvvPvQPvPvPPvPvPPvPvPvPvvPvPvrr")
LAST_ORDER = ("ooooQQRvvRQwvwvRwwooooQvRPvPvvPvPvPPvvPPvPvPPvwPPvPPwwPwPwPPwPPwPwwPPwPwwuuPPPoooo")
ANC = 17
NRM = 16
PART = ("HSR")

F32, BF16, I32 = jnp.float32, jnp.bfloat16, jnp.int32
NN = (((1,), (0,)), ((), ()))
NT = (((1,), (1,)), ((), ()))


def _dot(a, b, dims=NN):
    return lax.dot_general(a, b, dims, preferred_element_type=F32)


def _pack(x):
    return pltpu.bitcast(x.astype(BF16), I32)


def _unpack(x):
    return pltpu.bitcast(x, BF16)


def _cat(xs, axis):
    return xs[0] if len(xs) == 1 else lax.concatenate(xs, axis)


def _tree(fn, xs):
    while len(xs) > 1:
        xs = [fn(xs[i], xs[i + 1]) if i + 1 < len(xs) else xs[i] for i in range(0, len(xs), 2)]
    return xs[0]


def _cols(x):
    return [x[:, g * 128:(g + 1) * 128] for g in range(x.shape[1] // 128)]


def _fold(fn, x):
    return fn(x.reshape(x.shape[0] // 8, 8, x.shape[1]), axis=0)


def _digest(x, rows=8):
    for n in (4 * rows, 2 * rows, rows):
        x = x[:n] | x[-n:]
    return x


def _iota(shape, dim):
    return lax.broadcasted_iota(I32, shape, dim)


def _aligned(i, n):
    return i if isinstance(i, int) else pl.multiple_of(i, n)


def _loop(n, body):
    def trip(i, carry):
        body(i)

    lax.fori_loop(0, n, trip, None)


def _row_mean(x):
    c = _cols(x)
    return _tree(lax.add, [jnp.sum(c[i] + c[i + 4], axis=-1, keepdims=True) for i in range(4)]) * (1.0 / D)


def _phi(t):
    return jnp.maximum(t, 0.0) + jnp.exp(jnp.minimum(t, 0.0))


def _rcp(x):
    return pltpu.reciprocal(x, approx=False, full_range=False)


def _rotate_quarters(xs, sign):
    for bit in (1, 2):
        on = _iota(xs[0].shape, 1) & (DH * bit) != 0
        xs = [lax.select(on, xs[(i + sign * bit) % 4], xs[i]) for i in range(4)]
    return xs


def _rotate_rows(x, sign):
    n = x.shape[0] // 4
    return _cat(_rotate_quarters([x[i * n:(i + 1) * n] for i in range(4)], sign), 0)


def _exchange(xs):
    ys = _rotate_quarters(xs, 1)
    return [ys[-i % 4] for i in range(4)]


def _lhs7(block, put):
    a11 = block(0, 0)
    yield put((2, a11))
    a22 = block(1, 1)
    yield put((3, a22), (0, a11 + a22))
    a12 = block(0, 1)
    yield put((4, a11 + a12), (6, a12 - a22))
    a21 = block(1, 0)
    yield put((1, a21 + a22), (5, a21 - a11))


def _rhs7(b11, b12, b21, b22):
    return [b11 + b22, b11, b12 - b22, b21 - b11, b22, b11 + b12, b21 + b22]


def _strassen(prod, emit, park):
    m6 = prod(5)
    yield
    m2 = prod(1)
    park[0][...] = m6 - m2
    yield
    m4 = prod(3)
    emit(1, 0, m2 + m4)
    yield
    m1 = prod(0)
    c22 = park[0][...] + m1
    park[1][...] = m4 + m1
    yield
    m3 = prod(2)
    emit(1, 1, c22 + m3)
    yield
    m5 = prod(4)
    emit(0, 1, m3 + m5)
    c11 = park[1][...] - m5
    yield
    emit(0, 0, c11 + prod(6))
    yield


def _chain(*gens):
    for g in gens:
        yield from g


def _idle(n):
    for _ in range(n):
        yield


def _spaced(gen, *gaps):
    for i, x in enumerate(gen):
        yield x
        yield from _idle(gaps[i % len(gaps)] - 1)


def _merge(a, b):
    while True:
        xs = [x for x in (next(a, _merge), next(b, _merge)) if x is not _merge]
        if not xs:
            return
        xs = [x for x in xs if x is not None]
        yield _tree(lax.bitwise_or, xs) if xs else None


def _drain(gen):
    for _ in gen:
        pass


def _run(order, **gens):
    for ch in order.replace(" ", ""):
        next(gens[ch])
    for name, g in gens.items():
        assert next(g, _run) is _run, name


class _Buf:
    def __init__(self, ref, z):
        self.ref, self.z = ref, z

    def __setitem__(self, idx, val):
        self.ref[(0,) + (idx if isinstance(idx, tuple) else (idx,))] = val

    def __getitem__(self, idx):
        return self.ref[(self.z,) + (idx if isinstance(idx, tuple) else (idx,))]


def _kernel(x_hbm, wq_hbm, wk_hbm, wv_hbm, wo_hbm, beta_hbm, wqkv_hbm, wob_hbm, out_hbm,
            xin, xout, wa_raw, wqkv_raw, wob_raw, wa7, mem, gate, bias, ktail, vtail, scratch, zero, sems, beta):
    def panel_copy(m, n):
        src, col = ((wk_hbm, wq_hbm, wv_hbm)[m], n) if n < NP else (wo_hbm, 3 * (n - NP) + m)
        return pltpu.make_async_copy(src.at[:, pl.ds(col * 256, 256)], wa_raw.at[n, m],
                                     sems.at[SEM_PANEL + (2 + n if n else m)])

    def x_copy(i, n=1):
        return pltpu.make_async_copy(x_hbm.at[pl.ds(i, n)], xin.at[pl.ds(i, n)], sems.at[i])

    def wb_copy(m):
        return pltpu.make_async_copy(wqkv_hbm.at[:, pl.ds(_aligned(m * D, D), D)], wqkv_raw.at[m],
                                     sems.at[SEM_WB + m])

    def out_copy(*at):
        return pltpu.make_async_copy(xout.at[at], out_hbm.at[at], sems.at[SEM_OUT])

    beta_copy = pltpu.make_async_copy(beta_hbm, beta, sems.at[SEM_BETA])
    beta_copy.start()
    x_copy(0).start()
    for n in range(NP + 1):
        if n >= 2:
            wb_copy(n - 2).start()
        for m in range(3):
            panel_copy(m, n).start()
            if (m, n) == (1, 0):
                x_copy(1).start()
    last_copies = [panel_copy(0, NP + 1), pltpu.make_async_copy(wob_hbm, wob_raw, sems.at[SEM_OUT + 1]),
                   x_copy(2, 2)]
    for c in last_copies:
        c.start()
    x_copy(4, 4).start()

    def clear(i):
        zero[i] = 0
        mem[:, i] = jnp.zeros((2,) + mem.shape[2:], F32)
        for tail in (ktail, vtail):
            tail[:, pl.ds(2 * i, 2)] = jnp.zeros((2, 2, HALO, 128), F32)
        scratch["tmp"][0, 0, pl.ds(2 * i, 2)] = jnp.zeros((2, H * PITCH, 128), I32)
        scratch["ot"][1][0, i // 2, i % 2] = jnp.zeros((128, CH), F32)

    _loop(NP, clear)
    z = zero[1]
    st = jax.tree.map(lambda r: _Buf(r, z), scratch)
    ops, wb7, tmp, nxt, cur, qb, kb, vb = [st[k] for k in ("ops", "wb7", "tmp", "nxt", "cur", "qb", "kb", "vb")]

    def prep_rows(m, n, k):
        rows = [pl.ds(_aligned((2 * k + r) * CH, CH), CH) for r in range(2)]
        ws = _rhs7(*[w for r in rows for w in _cols(wa_raw[n, m, r, :].astype(F32))])
        out = _cols(_pack(_cat([ws[j] for j in (0, 2, 3, 5, 6)], 1)))
        out += [_pack(wa_raw[n + z, m, rows[r], pl.ds(r * 128, 128)]) for r in range(2)]
        for j, w in zip((0, 2, 3, 5, 6, 1, 4), out):
            wa7[m][n, j, pl.ds(_aligned(k * (CH // 2), CH // 2), CH // 2), :] = w
        return out

    def prep_panel(m, n):
        for k in range(NP):
            bits = _tree(lax.bitwise_or, prep_rows(m, n, k))
            for b in range(CH // 16):
                yield bits[8 * b:8 * b + 8]

    def wait_panels(n):
        pltpu.make_async_copy(wa_raw.at[n], wa_raw.at[n], sems.at[SEM_PANEL + 2 + n]).wait()

    def spread(m, j, g, w):
        w = _pack(w)
        for h in range(8):
            tmp[m, j, pl.ds((8 * g + h) * PITCH, DH // 2)] = w[h * DH // 2:(h + 1) * DH // 2]
        return w[-8:]

    def spread_qkv(m):
        for j in range(G):
            for g in range(NP):
                yield spread(m, j, g, wqkv_raw[m, pl.ds(j * 128, 128), pl.ds(g * 256, 256)].T)

    def gather(m, dst, slot=0):
        for k in range(2 * NP):
            ws = [_cat([tmp[m, j, pl.ds(k // 2 * 4 + k % 2 + 2 * r, H, stride=PITCH)] for j in range(s, G, 2)], 1)
                  for r in range(2) for s in range(2)]
            a, b, c, d = [lax.bitcast_convert_type(_cat([w << 16, w & -65536], 0), F32) for w in ws]
            ws = _pack(_cat(_rhs7(a, c, b, d) if dst < 2 else _rhs7(a, b, c, d), 0))
            wb7[dst][slot, :, pl.ds(k * H, H)] = ws.reshape(7, H, D // 2)
            bits = _cols(_digest(ws, H))
            for half in (bits[0] | bits[1], bits[2] | bits[3]):
                for row in (0, 16, 8, 24):
                    yield half[row:row + 8]

    recent, pending = [], []

    def streamed(y, slots=None):
        recent.extend((y, 16 * b) for b in range(slots or y.shape[0] // 16))

    def result(age):
        y, row = recent[-age]
        return y[row:row + 8, :128]

    def project(slot, rhs, emit, fill, dims=NN):
        def prod(i):
            rows, start = [], 0
            for b in range(CH // 16):
                mark = next(fill, None)
                while b == 0 and pending and pending[0][0] <= len(recent):
                    late = pending.pop(0)[1]
                    mark = late if mark is None else mark | late
                if mark is None:
                    continue
                if len(recent) >= 12 - b:
                    mark = mark | lax.bitcast_convert_type(result(12 - b), I32)
                if b > start:
                    rows.append(ops[slot][i, pl.ds(8 * start, 8 * (b - start))])
                    start = b
                ops[slot][7, pl.ds(8 * b, 8), pl.ds(0, 128)] = mark
            rows.append(ops[slot][i, pl.ds(8 * start, CH // 2 - 8 * start)])
            y = _dot(_unpack(_cat(rows, 0)), _unpack(rhs(i)), dims)
            streamed(y)
            return y

        return _strassen(prod, emit, st["park"])

    def done(fill):
        assert next(fill, done) is done
        recent.clear()
        pending.clear()

    def put_operand(slot, b, n):
        def put(*items):
            packed = _cols(_pack(_cat([a for _, a in items], 1)))
            for (i, _), a in zip(items, packed):
                ops[slot][i, pl.ds(8 * b, 8), pl.ds(n * 128, 128)] = a
            return _tree(lax.bitwise_or, packed)

        return put

    def put_chunk(slot, h):
        h, parts = _cols(h), []
        _drain(_lhs7(lambda r, s: _cat(h[s::2], 1)[r * CH:(r + 1) * CH], lambda *items: parts.extend(items)))
        packed = _pack(_cat([a for _, a in sorted(parts, key=lambda item: item[0])], 0))
        ops[slot][pl.ds(0, 7)] = packed.reshape(7, CH // 2, D // 2)
        return packed

    def norm(x, c, slot, gap):
        x, stat = st[x][c], st["stat"][c]
        for b in range(2 * CH // NRM):
            rows = pl.ds(NRM * b, NRM)
            v = x[rows]
            m = _row_mean(v)
            d = v - m
            stat[0, rows] = jnp.broadcast_to(m, (NRM, 128))
            stat[1, rows] = jnp.broadcast_to(lax.rsqrt(_row_mean(d * d) + 1e-5), (NRM, 128))

        def apply():
            h = (x[...] - _cat([stat[0]] * G, 1)) * _cat([stat[1]] * G, 1)
            bits = _cols(_digest(put_chunk(slot + c, h), CH // 2))
            bits = [bits[0] | bits[1], bits[2] | bits[3]]
            for b in range(CH // 16):
                for half in bits:
                    yield half[8 * b:8 * b + 8]

        return _chain(_idle(72), _spaced(apply(), 2 * gap))

    bias[...] = jnp.where(_iota((DH, CH), 0) > _iota((DH, CH), 1) % DH, NEG, 0.0)
    beta_copy.wait()
    b = jnp.broadcast_to(beta[...].astype(F32).reshape(1, H), (H, H))
    b = jnp.sum(jnp.where(_iota((H, H), 0) == _iota((H, H), 1), b, 0.0), axis=1, keepdims=True)
    gate[...] = jnp.broadcast_to(1.0 / (1.0 + jnp.exp(-b)), (H, 128)).reshape(NP, 8, 128)
    x_copy(0).wait()
    x = xin[0].astype(F32)
    st["xb"][0][...] = x
    d = x - jnp.mean(x, axis=-1, keepdims=True)
    put_chunk(HA, d * lax.rsqrt(jnp.mean(d * d, axis=-1, keepdims=True) + 1e-5))
    for m in range(3):
        panel_copy(m, 0).wait()
        _loop(NP, lambda k: prep_rows(m, 0, k))
        if m == 1:
            x_copy(1).wait()
            st["xb"][1][...] = xin[1].astype(F32)

    def step(it, carry):
        seg, pair = it // 2, it % 2

        def a_proj(m, n, c, fill):
            def emit(r, e, y):
                j = 2 * c + r
                if m == 0:
                    pk = _phi(y)
                    nxt["k"][e, j], nxt["pk"][e, j] = _cols(_pack(_cat([y, pk], 1)))
                    nxt["z"][e, j] = _fold(jnp.sum, pk)
                    return
                if m == 1:
                    y = _rotate_rows(y, -1)
                    nxt["pq"][e, j] = _pack(_phi(y))
                    y = y * QSCALE
                y = _pack(y.astype(BF16).T)
                nxt["qt" if m == 1 else "vt"][e, j] = y
                pending.append((len(recent) + 40, y[-8:]))

            return project(HA + c, lambda i: wa7[m][n, i], emit, fill)

        def a_recall(n):
            for e in range(2):
                r = _dot(mem[pair, n, e].astype(BF16), _unpack(nxt["pq"][e].reshape(L // 2, 128)), NT)
                st["r"][e][...] = r[:136]
                yield

        def a_update(n):
            row, head = _iota((144, 128), 0), _iota((144, 128), 1) // DH
            own = jnp.where(row < 128, row // DH, row - 128) == head
            for e in range(2):
                vt = _unpack(_cat([nxt["vt"][e, j] for j in range(NCH)], 1))
                zs = jnp.sum(jnp.sum(nxt["z"][e], axis=0), axis=0, keepdims=True)
                new = _cat([_dot(vt, _unpack(nxt["pk"][e].reshape(L // 2, 128))), jnp.broadcast_to(zs, (16, 128))], 0)
                mem[pair, n, e] = mem[pair, n, e] + jnp.where(own, new, 0.0)
                yield

        def a_scores(src, e):
            blank = jnp.zeros((DH // 2, CH), I32)
            quarter = (_iota((CH // 2, CH), 1) // DH - _iota((CH // 2, CH), 0) // (DH // 2)) & 3
            for j in range(NCH):
                qt = src["qt"][e, j]
                top = [None] * 4
                for t in reversed(range(4)):
                    sc = _dot(_unpack(src["k"][e, j, pl.ds(0, (t + 1) * DH // 2)]),
                              _unpack(jnp.where(quarter == t, qt, 0)))
                    sc = _cat([sc[:t * DH]] * (t > 0) + [sc[t * DH:] + bias[...]], 0)
                    st["s"][e][j][pl.ds(j * CH, (t + 1) * DH), pl.ds(t * CH, CH)] = sc
                    top[t] = _fold(jnp.max, sc)
                    if t == 3:
                        streamed(sc, 5)
                top = _cat(_exchange(top), 1)
                if j > 0:
                    heads = [_cat([qt[a * DH // 2:(a + 1) * DH // 2] if a == hh else blank for a in range(4)], 0)
                             for hh in range(4)]
                    sc = _dot(_unpack(src["k"][e, pl.ds(0, j)].reshape(j * CH // 2, 128)), _unpack(_cat(heads, 1)))
                    st["s"][e][j][pl.ds(0, j * CH)] = sc
                    top = jnp.maximum(top, _fold(jnp.max, sc))
                    streamed(sc)
                st["top"][e][j][pl.ds(0, 8)] = jnp.broadcast_to(jnp.max(top, axis=0, keepdims=True), (8, 4 * CH))
                yield

        def a_values(src, n, e):
            def tops(j):
                if len(recent) >= ANC:
                    st["top"][e][j][pl.ds(8, 8), pl.ds(0, 128)] = result(ANC)
                return _cols(st["top"][e][j][pl.ds(0, 8)])

            def probs(j, row, rows, col, top, l):
                p = jnp.exp2(st["s"][e][j][pl.ds(row, rows), pl.ds(col * CH, CH)] - _cat([top] * (rows // 8), 0))
                for a in reversed(range(rows // 16)):
                    l = p[16 * a:16 * a + 16] if l is None else l + p[16 * a:16 * a + 16]
                return p, _fold(jnp.sum, l)

            def mix(i, hh, p):
                return _dot(_unpack(src["vt"][e, i, pl.ds(hh * DH // 2, DH // 2)]), p.astype(BF16))

            def finish(j, hh, acc, l):
                g = gate[n, pl.ds(4 * e + hh, 1), :]
                rden = _rcp(st["r"][e][pl.ds(128 + hh, 1), pl.ds(j * CH, CH)] + 1e-6)
                rl = _rcp(jnp.sum(l, axis=0, keepdims=True))
                st["ot"][j // 2][j % 2, e, pl.ds(hh * DH, DH)] = (
                    acc * ((1.0 - g) * rl) + st["r"][e][pl.ds(hh * DH, DH), pl.ds(j * CH, CH)] * (g * rden))

            for j in range(NCH):
                p, l = zip(*[probs(j, j * CH, (t + 1) * DH, t, top, None)
                             for t, top in enumerate(_exchange(tops(j)))])
                l = _exchange(l)
                p = [_exchange([jnp.zeros((DH // 2, CH), I32)] * a
                               + _cols(_pack(_cat([p[t][a * DH:(a + 1) * DH] for t in range(a, 4)], 1))))
                     for a in range(4)]
                acc = [mix(j, hh, _unpack(_cat([p[a][hh] for a in range(4)], 0))) for hh in range(4)]
                if j == 0:
                    for hh in range(4):
                        finish(j, hh, acc[hh], l[hh])
                yield
                for hp in range(2):
                    for i in range(j):
                        top = tops(j)
                        for hh in (2 * hp, 2 * hp + 1):
                            p, more = probs(j, i * CH, CH, hh, top[hh], None)
                            acc[hh], l[hh] = acc[hh] + mix(i, hh, p), l[hh] + more
                            if i == j - 1:
                                finish(j, hh, acc[hh], l[hh])
                        yield

        def a_operands(n, c):
            col = _aligned(n * 128, 128)

            def put(*items):
                out = [_rotate_rows(_pack(a.astype(BF16).T), 1) for _, a in items]
                for (i, _), a in zip(items, out):
                    ops[OA + c][i, :, pl.ds(col, 128)] = a
                return _tree(lax.bitwise_or, [a[-8:] for a in out])

            return _lhs7(lambda r, e: st["ot"][c][r, e], put)

        def a_out(c, fill):
            for n in range(NP):
                def emit(r, s, y):
                    at = (pl.ds(r * CH, CH), pl.ds((2 * n + s) * 128, 128))
                    st["xa"][c][at] = st["xb"][c][at] + y

                yield from project(OA + c, lambda i: wa7[n % 3][NP + n // 3, i], emit, fill)

        def b_proj(c, m, fill):
            for n in range(NP):
                def emit(r, s, y):
                    if m == 0:
                        qb[c][2 * n + s, pl.ds(r * CH, CH)] = y * QSCALE
                    else:
                        (kb, vb)[m - 1][2 * n + s, pl.ds(HALO + (2 * c + r) * CH, CH)] = y

                _drain(project(HB + c, lambda i: wb7[m // 2][m % 2, i, pl.ds(n * CH // 2, CH // 2)], emit, fill, NT))

        def b_logits(c):
            for b in range(2 * CH // 16):
                t0 = 2 * c * CH + 16 * b
                q = qb[c][pl.ds(0, G), pl.ds(16 * b, 16)]
                for w in range(WIN):
                    a = jnp.sum(q * kb[:, pl.ds(HALO + t0 - DIL * w, 16)], axis=0)
                    a = (a + pltpu.roll(a, 64, 1)) + (pltpu.roll(a, 32, 1) + pltpu.roll(a, 96, 1))
                    if t0 < DIL * w:
                        a = jnp.where(_iota((16, 128), 0) + (seg * L + t0) >= DIL * w, a, NEG)
                    st["lb"][c][w, pl.ds(16 * b, 16)] = a

        def b_probs(c):
            a = st["lb"][c][:, pl.ds(0, 2 * CH)]
            p = jnp.exp2(a - jnp.max(a, axis=0, keepdims=True))
            qb[c][pl.ds(0, WIN), pl.ds(0, 2 * CH)] = p
            l = jnp.sum(p, axis=0)
            st["stat"][c][0] = _rcp(l)
            l = lax.bitcast_convert_type(l, I32)
            for b in range(2 * CH // 8):
                yield l[8 * b:8 * b + 8]

        def b_values(c):
            for b in range(CH // 16):
                for n in range(NP):
                    if len(recent) >= 16:
                        qb[c][WIN, pl.ds(0, 8)] = result(16)
                    o = []
                    for r in range(2):
                        rows = pl.ds(r * CH + 16 * b, 16)
                        t0 = HALO + (2 * c + r) * CH + 16 * b
                        v = _cat([vb[pl.ds(2 * n, 2), pl.ds(t0 - DIL * w, 16)] for w in range(WIN)], 1)
                        a = v.reshape(2, WIN, 16, 128) * qb[c][pl.ds(0, WIN), rows]
                        o.append(jnp.sum(a, axis=1) * st["stat"][c][0, rows])
                    yield from _lhs7(lambda r, s: o[r][s], put_operand(OB + c, b, n))

        def b_out(c, fill):
            following = 2 * jnp.minimum(seg + 1, NSEG - 1) + c
            for n in range(NP):
                def emit(r, s, y):
                    at = (pl.ds(r * CH, CH), pl.ds((2 * n + s) * 128, 128))
                    x = st["xa"][c][at] + y
                    xout[(2 * seg + c,) + at] = x.astype(BF16)
                    st["xb"][c][at] = jnp.where(pair == 1, xin[(following,) + at].astype(F32), x)

                for i, _ in enumerate(project(OB + c, lambda i: wb7[2][0, i, :, pl.ds(n * 128, 128)], emit, fill)):
                    if (c, n, i) == (1, 2, 1):
                        @pl.when(pair == 1)
                        def _():
                            out_copy(2 * seg).start()
                            out_copy(2 * seg + 1, slice(None), pl.ds(0, D // 2)).start()

        if "H" in PART:
            fill = norm("xb", 1, HA, 3)
            for c in range(2):
                for m in (2, 1, 0):
                    _drain(a_proj(m, 0, c, fill))
                done(fill)
            _drain(a_recall(0))

        def stage(n, extra):
            def keep(name):
                for e in range(2):
                    for j in range(NCH):
                        w = nxt[name][e, j]
                        cur[name][e, j] = w
                        yield _digest(w)

            fill = _merge(extra, _chain(
                keep("k"), keep("qt"), keep("vt"), _idle(8), _spaced(a_operands(jnp.maximum(n - 1, 0), 1), 8),
                _idle(192), _spaced(a_operands(n, 0), 8)))
            _run(STAGE_ORDER, P=_chain(*[a_proj(m, n + 1, c, fill) for m in (2, 1, 0) for c in range(2)]),
                 Q=_chain(a_scores(cur, 0), a_scores(cur, 1)), v=_chain(a_values(cur, n, 0), a_values(cur, n, 1)),
                 u=a_update(n), r=a_recall(n + 1))
            done(fill)

        def prepare(n):
            prev = jnp.maximum(n - 1, 0)
            yield from _spaced(gather(prev, 0, prev), 3, 3, 2)
            yield from _idle(5)
            wb_copy(n).wait()
            wait_panels(n + 2)
            yield from _merge(_chain(_idle(16), _spaced(spread_qkv(n), 4)),
                              _spaced(_chain(*[prep_panel(m, n + 2) for m in (0, 2, 1)]), 1, 2, 2))

        @pl.when(it == 0)
        def _():
            wait_panels(1)
            _loop(NP, lambda k: [prep_rows(m, 1, k) for m in range(3)])
            _loop(NP - 1, lambda n: stage(n, prepare(n)))
            for c in last_copies:
                c.wait()

            def last(k):
                prep_rows(0, NP + 1, k)
                for j in range(G):
                    spread(3, j, k, wob_raw[pl.ds(_aligned(k * 256, 256), 256), pl.ds(j * 128, 128)])

            _loop(NP, last)

        @pl.when(it > 0)
        def _():
            _loop(NP - 1, lambda n: stage(n, _idle(0)))

        if "R" not in PART:
            xout[0, :16, :128] = _unpack(tmp[0, 0, :8] | ops[OA][0, :8, :128] | ops[OA + 1][0, :8, :128] | wb7[0][0, 0, :8, :128])
            return carry

        pl.when(it == 1)(x_copy(4, 4).wait)
        kb[:, pl.ds(0, HALO)] = ktail[pair]
        vb[:, pl.ds(0, HALO)] = vtail[pair]
        _run(LAST_ORDER, Q=a_scores(nxt, 0), R=a_scores(nxt, 1), v=a_values(nxt, NP - 1, 0),
             w=a_values(nxt, NP - 1, 1), u=a_update(NP - 1),
             P=a_out(0, _idle(0)),
             o=_chain(a_operands(NP - 2, 1), a_operands(NP - 1, 0), a_operands(NP - 1, 1)))
        fill = norm("xa", 0, HB, 4)
        _drain(a_out(1, fill))
        done(fill)
        if "T" in PART:
            xout[0, :16, :128] = _unpack(ops[HB][0, :8, :128] | _pack(st["xa"][1][:16, :128]))
            return carry
        for c in range(2):
            if c == 0:
                fill = _chain(norm("xa", 1, HB, 4), _spaced(gather(2, 1), 4, 4, 3))
            else:
                fill = _chain(_idle(12), _spaced(b_values(0), 1, 2, 2), _spaced(gather(3, 2), 3, 3, 4))
            b_proj(c, 0, fill)
            b_proj(c, 1, fill)
            done(fill)
            b_logits(c)
            fill = _chain(_idle(156), _spaced(b_probs(c), 2))
            b_proj(c, 2, fill)
            done(fill)
        fill = _chain(_idle(12), _spaced(b_values(1), 2, 1, 2, 2, 1))
        b_out(0, fill)
        done(fill)
        fill = norm("xb", 0, HA, 4)
        b_out(1, fill)
        done(fill)
        ktail[pair] = kb[:, pl.ds(L, HALO)]
        vtail[pair] = vb[:, pl.ds(L, HALO)]
        pl.when(pair == 1)(out_copy(2 * seg + 1, slice(None), pl.ds(D // 2, D // 2)).start)
        return carry

    lax.fori_loop(0, 2 * NSEG, step, 0)
    pltpu.make_async_copy(xout, out_hbm, sems.at[SEM_OUT]).wait()


@jax.jit
def pallas_interleave_layers__memory_aug_infini_attn__sliding_local_dilated__prompt_kernel(
    A_x, A_wq, A_wk, A_wv, A_wo, A_beta, B_x, B_wqkv, B_wo,
):
    del B_x
    hbm = pl.BlockSpec(memory_space=pl.ANY)
    vm = pltpu.VMEM
    chunks = (2 * NSEG, 2 * CH, D)
    heads = vm((1, 2, NCH, CH // 2, 128), I32)
    scratch = dict(
        ops=[vm((1, 8, CH // 2, D // 2), I32)] * 8,
        wb7=[vm((1, n, 7, D // 4, D // 2), I32) for n in (2, 1, 1)],
        tmp=vm((1, 4, G, H * PITCH, 128), I32),
        park=[vm((1, CH, 128), F32)] * 2,
        stat=[vm((1, 2, 2 * CH, 128), F32)] * 2,
        xa=[vm((1, 2 * CH, D), F32)] * 2,
        xb=[vm((1, 2 * CH, D), F32)] * 2,
        nxt=dict(k=heads, qt=heads, vt=heads, pk=heads, pq=heads, z=vm((1, 2, NCH, 8, 128), F32)),
        cur=dict(k=heads, qt=heads, vt=heads),
        s=[[vm((1, (j + 1) * CH, 4 * CH), F32) for j in range(NCH)]] * 2,
        top=[[vm((1, 16, 4 * CH), F32)] * NCH] * 2,
        r=[vm((1, 136, L), F32)] * 2,
        ot=[vm((1, 2, 2, 128, CH), F32)] * 2,
        qb=[vm((1, G + 4, 2 * CH + 8, 128), F32)] * 2,
        lb=[vm((1, WIN, 2 * CH + 8, 128), F32)] * 2,
        kb=vm((1, G, HALO + L + 24, 128), F32),
        vb=vm((1, G, HALO + L + 24, 128), F32),
    )
    out = pl.pallas_call(
        _kernel,
        name="infini_dilated",
        out_shape=jax.ShapeDtypeStruct(chunks, BF16),
        in_specs=[hbm] * 8,
        out_specs=hbm,
        scratch_shapes=[
            vm(chunks, BF16), vm(chunks, BF16),
            vm((NP + 2, 3, D, 256), BF16), vm((3, D, D), BF16), vm((D, D), BF16),
            [vm((NP + 1 + (m == 0), 7, D // 4, 128), I32) for m in range(3)],
            vm((2, NP, 2, 144, 128), F32), vm((NP, 8, 128), F32), vm((DH, CH), F32),
            vm((2, G, HALO, 128), F32), vm((2, G, HALO, 128), F32),
            scratch, pltpu.SMEM((NP,), I32), pltpu.SemaphoreType.DMA((SEM_OUT + 2,)), vm((H,), BF16),
        ],
        compiler_params=pltpu.CompilerParams(vmem_limit_bytes=110 * 2 ** 20),
    )(A_x.reshape(chunks), A_wq, A_wk, A_wv, A_wo, A_beta, B_wqkv, B_wo)
    return out.reshape(A_x.shape)
```

```python
import math

import jax
import jax.numpy as jnp
from jax import lax
import jax.experimental.pallas as pl
import jax.experimental.pallas.tpu as pltpu

S = 2048
D = 1024
H = 32
DH = D // H
NSEG = 4
L = S // NSEG
WIN, DIL = 8, 2
HALO = 16
G = D // 128
NP = G // 2
CH = 128
NCH = L // CH
PITCH = DH // 2 + 1
QSCALE = DH ** -0.5 * math.log2(math.e)
NEG = -1e9
HA, OA, HB, OB = 0, 2, 4, 6
SEM_BETA, SEM_WB, SEM_PANEL, SEM_WOB, SEM_OUT = 3, 5, 8, 16, 17

STAGE_ORDER = "uuPPQQPPPvPPvQPvPvPvPQPvPvvPPvvPPvQQPPvPvvPvPvPPvPPPvQPPvvPvQPvPvPPvPvPPvPvPvPvvPvPvrr"
FIRST_ORDER = "uPuPPPQQPvPvPQPvPvPPvQPvvPvPPvvPPQQPvPPPvvvvPvPPvPPPvQPPvvPPvPQPvvPvPPvPvPvPvPvvPvPvrr"
LAST_ORDER = "ooooQQRvvRQwvwvRwwooooQvRPvPvvvPvPPPPvvPvPvPvwPPPvPPwPwwwPPwPPPwPPwwPwPwwuuPPPoooo"

F32, BF16, I32 = jnp.float32, jnp.bfloat16, jnp.int32
NN = (((1,), (0,)), ((), ()))
NT = (((1,), (1,)), ((), ()))


def _dot(a, b, dims=NN):
    return lax.dot_general(a, b, dims, preferred_element_type=F32)


def _pack(x):
    return pltpu.bitcast(x.astype(BF16), I32)


def _unpack(x):
    return pltpu.bitcast(x, BF16)


def _cat(xs, axis):
    return xs[0] if len(xs) == 1 else lax.concatenate(xs, axis)


def _tree(fn, xs):
    while len(xs) > 1:
        xs = [fn(xs[i], xs[i + 1]) if i + 1 < len(xs) else xs[i] for i in range(0, len(xs), 2)]
    return xs[0]


def _cols(x):
    return [x[:, g * 128:(g + 1) * 128] for g in range(x.shape[1] // 128)]


def _fold(fn, x):
    return fn(x.reshape(x.shape[0] // 8, 8, x.shape[1]), axis=0)


def _digest(x, rows=8):
    for n in (4 * rows, 2 * rows, rows):
        x = x[:n] | x[-n:]
    return x


def _iota(shape, dim):
    return lax.broadcasted_iota(I32, shape, dim)


def _aligned(i, n):
    return i if isinstance(i, int) else pl.multiple_of(i, n)


def _loop(n, body):
    def trip(i, carry):
        body(i)

    lax.fori_loop(0, n, trip, None)


def _row_mean(x):
    c = _cols(x)
    return _tree(lax.add, [jnp.sum(c[i] + c[i + 4], axis=-1, keepdims=True) for i in range(4)]) * (1.0 / D)


def _phi(t):
    return jnp.maximum(t, 0.0) + jnp.exp(jnp.minimum(t, 0.0))


def _rcp(x):
    return pltpu.reciprocal(x, approx=False, full_range=False)


def _rotate_quarters(xs, sign):
    for bit in (1, 2):
        on = _iota(xs[0].shape, 1) & (DH * bit) != 0
        xs = [lax.select(on, xs[(i + sign * bit) % 4], xs[i]) for i in range(4)]
    return xs


def _rotate_rows(x, sign):
    n = x.shape[0] // 4
    return _cat(_rotate_quarters([x[i * n:(i + 1) * n] for i in range(4)], sign), 0)


def _exchange(xs):
    ys = _rotate_quarters(xs, 1)
    return [ys[-i % 4] for i in range(4)]


def _lhs7(block, put):
    a11 = block(0, 0)
    yield put((2, a11))
    a22 = block(1, 1)
    yield put((3, a22), (0, a11 + a22))
    a12 = block(0, 1)
    yield put((4, a11 + a12), (6, a12 - a22))
    a21 = block(1, 0)
    yield put((1, a21 + a22), (5, a21 - a11))


def _rhs7(b11, b12, b21, b22):
    return [b11 + b22, b11, b12 - b22, b21 - b11, b22, b11 + b12, b21 + b22]


def _strassen(prod, emit, park):
    m6 = prod(5)
    yield
    m2 = prod(1)
    park[0][...] = m6 - m2
    yield
    m4 = prod(3)
    emit(1, 0, m2 + m4)
    yield
    m1 = prod(0)
    c22 = park[0][...] + m1
    park[1][...] = m4 + m1
    yield
    m3 = prod(2)
    emit(1, 1, c22 + m3)
    yield
    m5 = prod(4)
    emit(0, 1, m3 + m5)
    c11 = park[1][...] - m5
    yield
    emit(0, 0, c11 + prod(6))
    yield


def _chain(*gens):
    for g in gens:
        yield from g


def _idle(n):
    for _ in range(n):
        yield


def _spaced(gen, *gaps):
    for i, x in enumerate(gen):
        yield x
        yield from _idle(gaps[i % len(gaps)] - 1)


def _merge(a, b):
    while True:
        xs = [x for x in (next(a, _merge), next(b, _merge)) if x is not _merge]
        if not xs:
            return
        xs = [x for x in xs if x is not None]
        yield _tree(lax.bitwise_or, xs) if xs else None


def _drain(gen):
    for _ in gen:
        pass


def _run(order, **gens):
    for ch in order.replace(" ", ""):
        next(gens[ch])
    for name, g in gens.items():
        assert next(g, _run) is _run, name


class _Buf:
    def __init__(self, ref, z):
        self.ref, self.z = ref, z

    def __setitem__(self, idx, val):
        self.ref[(0,) + (idx if isinstance(idx, tuple) else (idx,))] = val

    def __getitem__(self, idx):
        return self.ref[(self.z,) + (idx if isinstance(idx, tuple) else (idx,))]


def _kernel(x_hbm, wq_hbm, wk_hbm, wv_hbm, wo_hbm, beta_hbm, wqkv_hbm, wob_hbm, out_hbm,
            xin, xout, wa_raw, wqkv_raw, wob_raw, wa7, mem, gate, bias, ktail, vtail, scratch, zero, sems, beta):
    def panel_copy(m, n):
        src, col = ((wk_hbm, wq_hbm, wv_hbm)[m], n) if n < NP else (wo_hbm, 3 * (n - NP) + m)
        return pltpu.make_async_copy(src.at[:, pl.ds(col * 256, 256)], wa_raw.at[n, m],
                                     sems.at[SEM_PANEL + (2 + n if n else m)])

    def x_copy(i, n=1):
        return pltpu.make_async_copy(x_hbm.at[pl.ds(i, n)], xin.at[pl.ds(i, n)], sems.at[i])

    def wb_copy(m):
        return pltpu.make_async_copy(wqkv_hbm.at[:, pl.ds(_aligned(m * D, D), D)], wqkv_raw.at[m],
                                     sems.at[SEM_WB + m])

    def out_copy(*at):
        return pltpu.make_async_copy(xout.at[at], out_hbm.at[at], sems.at[SEM_OUT])

    beta_copy = pltpu.make_async_copy(beta_hbm, beta, sems.at[SEM_BETA])
    beta_copy.start()
    x_copy(0).start()
    for n in range(NP + 1):
        if n >= 2:
            wb_copy(n - 2).start()
        for m in range(3):
            panel_copy(m, n).start()
            if (m, n) == (1, 0):
                x_copy(1).start()
    last_copies = [panel_copy(0, NP + 1), pltpu.make_async_copy(wob_hbm, wob_raw, sems.at[SEM_WOB]),
                   x_copy(2, 2)]
    for c in last_copies:
        c.start()
    x_copy(4, 4).start()

    def clear(i):
        zero[i] = 0
        mem[:, i] = jnp.zeros((2,) + mem.shape[2:], F32)
        for tail in (ktail, vtail):
            tail[:, pl.ds(2 * i, 2)] = jnp.zeros((2, 2, HALO, 128), F32)
        scratch["tmp"][0, 0, pl.ds(2 * i, 2)] = jnp.zeros((2, H * PITCH + 32, 128), I32)
        scratch["ot"][1][0, i // 2, i % 2] = jnp.zeros((128, CH), F32)

    _loop(NP, clear)
    z = zero[1]
    st = jax.tree.map(lambda r: _Buf(r, z), scratch)
    ops, wb7, tmp, nxt, cur, qb, kb, vb = [st[k] for k in ("ops", "wb7", "tmp", "nxt", "cur", "qb", "kb", "vb")]

    def prep_rows(m, n, k):
        rows = [pl.ds(_aligned((2 * k + r) * CH, CH), CH) for r in range(2)]
        ws = _rhs7(*[w for r in rows for w in _cols(wa_raw[n, m, r, :].astype(F32))])
        out = _cols(_pack(_cat([ws[j] for j in (0, 2, 3, 5, 6)], 1)))
        out += [_pack(wa_raw[n + z, m, rows[r], pl.ds(r * 128, 128)]) for r in range(2)]
        for j, w in zip((0, 2, 3, 5, 6, 1, 4), out):
            wa7[m][n, j, pl.ds(_aligned(k * (CH // 2), CH // 2), CH // 2), :] = w
        return out

    def prep_panel(m, n):
        for k in range(NP):
            bits = _tree(lax.bitwise_or, prep_rows(m, n, k))
            for b in range(CH // 16):
                yield bits[8 * b:8 * b + 8]

    def wait_panels(n):
        pltpu.make_async_copy(wa_raw.at[n], wa_raw.at[n], sems.at[SEM_PANEL + 2 + n]).wait()

    def spread(m, j, g, w):
        w = _pack(w)
        for h in range(8):
            tmp[m, j, pl.ds((8 * g + h) * PITCH, DH // 2)] = w[h * DH // 2:(h + 1) * DH // 2]
        return w[-8:]

    def spread_qkv(m):
        for j in range(G):
            for g in range(NP):
                yield spread(m, j, g, wqkv_raw[m, pl.ds(j * 128, 128), pl.ds(g * 256, 256)].T)

    def gather(m, dst, slot=0):
        for k in range(2 * NP):
            ws = [_cat([tmp[m, j, pl.ds(k // 2 * 4 + k % 2 + 2 * r, H, stride=PITCH)] for j in range(s, G, 2)], 1)
                  for r in range(2) for s in range(2)]
            a, b, c, d = [lax.bitcast_convert_type(_cat([w << 16, w & -65536], 0), F32) for w in ws]
            ws = _pack(_cat(_rhs7(a, c, b, d) if dst < 2 else _rhs7(a, b, c, d), 0))
            wb7[dst][slot, :, pl.ds(k * H, H)] = ws.reshape(7, H, D // 2)
            bits = _cols(_digest(ws, H))
            for half in (bits[0] | bits[1], bits[2] | bits[3]):
                for row in (0, 16, 8, 24):
                    yield half[row:row + 8]

    recent, pending = [], []

    def streamed(y, slots=None):
        recent.extend((y, 16 * b) for b in range(slots or y.shape[0] // 16))

    def result(age):
        y, row = recent[-age]
        return y[row:row + 8, :128]

    def project(slot, rhs, emit, fill, dims=NN):
        def prod(i):
            rows, start = [], 0
            for b in range(CH // 16):
                mark = next(fill, None)
                while b == 0 and pending and pending[0][0] <= len(recent):
                    late = pending.pop(0)[1]
                    mark = late if mark is None else mark | late
                if mark is None:
                    continue
                if len(recent) >= 12 - b:
                    mark = mark | lax.bitcast_convert_type(result(12 - b), I32)
                if b > start:
                    rows.append(ops[slot][i, pl.ds(8 * start, 8 * (b - start))])
                    start = b
                ops[slot][7, pl.ds(8 * b, 8), pl.ds(0, 128)] = mark
            rows.append(ops[slot][i, pl.ds(8 * start, CH // 2 - 8 * start)])
            y = _dot(_unpack(_cat(rows, 0)), _unpack(rhs(i)), dims)
            streamed(y)
            return y

        return _strassen(prod, emit, st["park"])

    def done(fill):
        assert next(fill, done) is done
        recent.clear()
        pending.clear()

    def put_operand(slot, b, n):
        def put(*items):
            packed = _cols(_pack(_cat([a for _, a in items], 1)))
            for (i, _), a in zip(items, packed):
                ops[slot][i, pl.ds(8 * b, 8), pl.ds(n * 128, 128)] = a
            return _tree(lax.bitwise_or, packed)

        return put

    def put_chunk(slot, h):
        h, parts = _cols(h), []
        _drain(_lhs7(lambda r, s: _cat(h[s::2], 1)[r * CH:(r + 1) * CH], lambda *items: parts.extend(items)))
        packed = _pack(_cat([a for _, a in sorted(parts, key=lambda item: item[0])], 0))
        ops[slot][pl.ds(0, 7)] = packed.reshape(7, CH // 2, D // 2)
        return packed

    def norm(x, c, slot, gap):
        x, stat = st[x][c], st["stat"][c]
        for b in range(2 * CH // 16):
            rows = pl.ds(16 * b, 16)
            v = x[rows]
            m = _row_mean(v)
            d = v - m
            stat[0, rows] = jnp.broadcast_to(m, (16, 128))
            stat[1, rows] = jnp.broadcast_to(lax.rsqrt(_row_mean(d * d) + 1e-5), (16, 128))

        def apply():
            h = (x[...] - _cat([stat[0]] * G, 1)) * _cat([stat[1]] * G, 1)
            bits = _cols(_digest(put_chunk(slot + c, h), CH // 2))
            bits = [bits[0] | bits[1], bits[2] | bits[3]]
            for b in range(CH // 16):
                for half in bits:
                    yield half[8 * b:8 * b + 8]

        return _chain(_idle(72), _spaced(apply(), gap))

    bias[...] = jnp.where(_iota((DH, CH), 0) > _iota((DH, CH), 1) % DH, NEG, 0.0)
    beta_copy.wait()
    b = jnp.broadcast_to(beta[...].astype(F32).reshape(1, H), (H, H))
    b = jnp.sum(jnp.where(_iota((H, H), 0) == _iota((H, H), 1), b, 0.0), axis=1, keepdims=True)
    gate[...] = jnp.broadcast_to(1.0 / (1.0 + jnp.exp(-b)), (H, 128)).reshape(NP, 8, 128)
    x_copy(0).wait()
    x = xin[0].astype(F32)
    st["xb"][0][...] = x
    d = x - jnp.mean(x, axis=-1, keepdims=True)
    put_chunk(HA, d * lax.rsqrt(jnp.mean(d * d, axis=-1, keepdims=True) + 1e-5))
    for m in range(3):
        panel_copy(m, 0).wait()
        _loop(NP, lambda k: prep_rows(m, 0, k))
        if m == 1:
            x_copy(1).wait()
            st["xb"][1][...] = xin[1].astype(F32)

    def step(it):
        seg, pair = it // 2, it % 2

        def a_proj(m, n, c, fill):
            def emit(r, e, y):
                j = 2 * c + r
                if m == 0:
                    pk = _phi(y)
                    nxt["k"][e, j], nxt["pk"][e, j] = _cols(_pack(_cat([y, pk], 1)))
                    nxt["z"][e, j] = _fold(jnp.sum, pk)
                    return
                if m == 1:
                    y = _rotate_rows(y, -1)
                    nxt["pq"][e, j] = _pack(_phi(y))
                    y = y * QSCALE
                y = _pack(y.astype(BF16).T)
                nxt["qt" if m == 1 else "vt"][e, j] = y
                pending.append((len(recent) + 40, y[-8:]))

            return project(HA + c, lambda i: wa7[m][n, i], emit, fill)

        def a_recall(n):
            for e in range(2):
                r = _dot(mem[pair, n, e].astype(BF16), _unpack(nxt["pq"][e].reshape(L // 2, 128)), NT)
                st["r"][e][...] = r[:136]
                yield

        def a_update(n):
            row, head = _iota((144, 128), 0), _iota((144, 128), 1) // DH
            own = jnp.where(row < 128, row // DH, row - 128) == head
            for e in range(2):
                vt = _unpack(_cat([nxt["vt"][e, j] for j in range(NCH)], 1))
                zs = jnp.sum(jnp.sum(nxt["z"][e], axis=0), axis=0, keepdims=True)
                new = _cat([_dot(vt, _unpack(nxt["pk"][e].reshape(L // 2, 128))), jnp.broadcast_to(zs, (16, 128))], 0)
                mem[pair, n, e] = mem[pair, n, e] + jnp.where(own, new, 0.0)
                yield

        def a_scores(src, e):
            blank = jnp.zeros((DH // 2, CH), I32)
            quarter = (_iota((CH // 2, CH), 1) // DH - _iota((CH // 2, CH), 0) // (DH // 2)) & 3
            for j in range(NCH):
                qt = src["qt"][e, j]
                top = [None] * 4
                for t in reversed(range(4)):
                    sc = _dot(_unpack(src["k"][e, j, pl.ds(0, (t + 1) * DH // 2)]),
                              _unpack(jnp.where(quarter == t, qt, 0)))
                    sc = _cat([sc[:t * DH]] * (t > 0) + [sc[t * DH:] + bias[...]], 0)
                    st["s"][e][j][pl.ds(j * CH, (t + 1) * DH), pl.ds(t * CH, CH)] = sc
                    top[t] = _fold(jnp.max, sc)
                    if t == 3:
                        streamed(sc, 5)
                top = _cat(_exchange(top), 1)
                if j > 0:
                    heads = [_cat([qt[a * DH // 2:(a + 1) * DH // 2] if a == hh else blank for a in range(4)], 0)
                             for hh in range(4)]
                    sc = _dot(_unpack(src["k"][e, pl.ds(0, j)].reshape(j * CH // 2, 128)), _unpack(_cat(heads, 1)))
                    st["s"][e][j][pl.ds(0, j * CH)] = sc
                    top = jnp.maximum(top, _fold(jnp.max, sc))
                    streamed(sc)
                st["top"][e][j][pl.ds(0, 8)] = jnp.broadcast_to(jnp.max(top, axis=0, keepdims=True), (8, 4 * CH))
                yield

        def a_values(src, n, e):
            def tops(j):
                if len(recent) >= 17:
                    st["top"][e][j][pl.ds(8, 8), pl.ds(0, 128)] = result(17)
                return _cols(st["top"][e][j][pl.ds(0, 8)])

            def probs(j, row, rows, col, top):
                p = jnp.exp2(st["s"][e][j][pl.ds(row, rows), pl.ds(col * CH, CH)] - _cat([top] * (rows // 8), 0))
                l = p[-16:]
                for a in reversed(range(rows // 16 - 1)):
                    l = l + p[16 * a:16 * a + 16]
                return p, _fold(jnp.sum, l)

            def mix(i, hh, p):
                return _dot(_unpack(src["vt"][e, i, pl.ds(hh * DH // 2, DH // 2)]), p.astype(BF16))

            def finish(j, hh, acc, l):
                g = gate[n, pl.ds(4 * e + hh, 1), :]
                rden = _rcp(st["r"][e][pl.ds(128 + hh, 1), pl.ds(j * CH, CH)] + 1e-6)
                rl = _rcp(jnp.sum(l, axis=0, keepdims=True))
                st["ot"][j // 2][j % 2, e, pl.ds(hh * DH, DH)] = (
                    acc * ((1.0 - g) * rl) + st["r"][e][pl.ds(hh * DH, DH), pl.ds(j * CH, CH)] * (g * rden))

            for j in range(NCH):
                p, l = zip(*[probs(j, j * CH, (t + 1) * DH, t, top)
                             for t, top in enumerate(_exchange(tops(j)))])
                l = _exchange(l)
                p = [_exchange([jnp.zeros((DH // 2, CH), I32)] * a
                               + _cols(_pack(_cat([p[t][a * DH:(a + 1) * DH] for t in range(a, 4)], 1))))
                     for a in range(4)]
                acc = [mix(j, hh, _unpack(_cat([p[a][hh] for a in range(4)], 0))) for hh in range(4)]
                if j == 0:
                    for hh in range(4):
                        finish(j, hh, acc[hh], l[hh])
                yield
                for hp in range(2):
                    for i in range(j):
                        top = tops(j)
                        for hh in (2 * hp, 2 * hp + 1):
                            p, more = probs(j, i * CH, CH, hh, top[hh])
                            acc[hh], l[hh] = acc[hh] + mix(i, hh, p), l[hh] + more
                            if i == j - 1:
                                finish(j, hh, acc[hh], l[hh])
                        yield

        def a_operands(n, c):
            col = _aligned(n * 128, 128)

            def put(*items):
                out = [_rotate_rows(_pack(a.astype(BF16).T), 1) for _, a in items]
                for (i, _), a in zip(items, out):
                    ops[OA + c][i, :, pl.ds(col, 128)] = a
                return _tree(lax.bitwise_or, [a[-8:] for a in out])

            return _lhs7(lambda r, e: st["ot"][c][r, e], put)

        def a_out(c, fill):
            for n in range(NP):
                def emit(r, s, y):
                    at = (pl.ds(r * CH, CH), pl.ds((2 * n + s) * 128, 128))
                    st["xa"][c][at] = st["xb"][c][at] + y

                yield from project(OA + c, lambda i: wa7[n % 3][NP + n // 3, i], emit, fill)

        def b_proj(c, m, fill):
            for n in range(NP):
                def emit(r, s, y):
                    if m == 0:
                        qb[c][2 * n + s, pl.ds(r * CH, CH)] = y * QSCALE
                    else:
                        (kb, vb)[m - 1][2 * n + s, pl.ds(HALO + (2 * c + r) * CH, CH)] = y

                _drain(project(HB + c, lambda i: wb7[m // 2][m % 2, i, pl.ds(n * CH // 2, CH // 2)], emit, fill, NT))

        def b_logits(c):
            for b in range(2 * CH // 16):
                t0 = 2 * c * CH + 16 * b
                q = qb[c][pl.ds(0, G), pl.ds(16 * b, 16)]
                for w in range(WIN):
                    a = jnp.sum(q * kb[:, pl.ds(HALO + t0 - DIL * w, 16)], axis=0)
                    a = (a + pltpu.roll(a, 64, 1)) + (pltpu.roll(a, 32, 1) + pltpu.roll(a, 96, 1))
                    if t0 < DIL * w:
                        a = jnp.where(_iota((16, 128), 0) + (seg * L + t0) >= DIL * w, a, NEG)
                    st["lb"][c][w, pl.ds(16 * b, 16)] = a

        def b_probs(c):
            a = st["lb"][c][:, pl.ds(0, 2 * CH)]
            p = jnp.exp2(a - jnp.max(a, axis=0, keepdims=True))
            qb[c][pl.ds(0, WIN), pl.ds(0, 2 * CH)] = p
            l = jnp.sum(p, axis=0)
            st["stat"][c][0] = _rcp(l)
            l = lax.bitcast_convert_type(l, I32)
            for b in range(2 * CH // 8):
                yield l[8 * b:8 * b + 8]

        def b_values(c):
            for b in range(CH // 16):
                for n in range(NP):
                    if len(recent) >= 16:
                        qb[c][WIN, pl.ds(0, 8)] = result(16)
                    o = []
                    for r in range(2):
                        rows = pl.ds(r * CH + 16 * b, 16)
                        t0 = HALO + (2 * c + r) * CH + 16 * b
                        v = _cat([vb[pl.ds(2 * n, 2), pl.ds(t0 - DIL * w, 16)] for w in range(WIN)], 1)
                        a = v.reshape(2, WIN, 16, 128) * qb[c][pl.ds(0, WIN), rows]
                        o.append(jnp.sum(a, axis=1) * st["stat"][c][0, rows])
                    yield from _lhs7(lambda r, s: o[r][s], put_operand(OB + c, b, n))

        def b_out(c, fill):
            following = 2 * jnp.minimum(seg + 1, NSEG - 1) + c
            for n in range(NP):
                def emit(r, s, y):
                    at = (pl.ds(r * CH, CH), pl.ds((2 * n + s) * 128, 128))
                    x = st["xa"][c][at] + y
                    xout[(2 * seg + c,) + at] = x.astype(BF16)
                    st["xb"][c][at] = jnp.where(pair == 1, xin[(following,) + at].astype(F32), x)

                for i, _ in enumerate(project(OB + c, lambda i: wb7[2][0, i, :, pl.ds(n * 128, 128)], emit, fill)):
                    if (c, n, i) == (1, 2, 1):
                        @pl.when(pair == 1)
                        def _():
                            out_copy(2 * seg).start()
                            out_copy(2 * seg + 1, slice(None), pl.ds(0, D // 2)).start()

        fill = norm("xb", 1, HA, 6)
        for c in range(2):
            for m in (2, 1, 0):
                _drain(a_proj(m, 0, c, fill))
            done(fill)
        _drain(a_recall(0))

        def stage(n, order, extra):
            def keep(name):
                for e in range(2):
                    for j in range(NCH):
                        w = nxt[name][e, j]
                        cur[name][e, j] = w
                        yield _digest(w)

            fill = _merge(extra, _chain(
                keep("k"), keep("qt"), keep("vt"), _idle(8), _spaced(a_operands(jnp.maximum(n - 1, 0), 1), 8),
                _idle(192), _spaced(a_operands(n, 0), 8)))
            _run(order, P=_chain(*[a_proj(m, n + 1, c, fill) for m in (2, 1, 0) for c in range(2)]),
                 Q=_chain(a_scores(cur, 0), a_scores(cur, 1)), v=_chain(a_values(cur, n, 0), a_values(cur, n, 1)),
                 u=a_update(n), r=a_recall(n + 1))
            done(fill)

        def prepare(n):
            prev = jnp.maximum(n - 1, 0)
            yield from _spaced(gather(prev, 0, prev), 3, 3, 2)
            yield from _idle(5)
            wb_copy(n).wait()
            wait_panels(n + 2)
            yield from _merge(_chain(_idle(16), _spaced(spread_qkv(n), 4)),
                              _spaced(_chain(*[prep_panel(m, n + 2) for m in (0, 2, 1)]), 1, 2, 2))

        @pl.when(it == 0)
        def _():
            wait_panels(1)
            _loop(NP, lambda k: [prep_rows(m, 1, k) for m in range(3)])
            _loop(NP - 1, lambda n: stage(n, FIRST_ORDER, prepare(n)))
            for c in last_copies:
                c.wait()

            def last(k):
                prep_rows(0, NP + 1, k)
                for j in range(G):
                    spread(3, j, k, wob_raw[pl.ds(_aligned(k * 256, 256), 256), pl.ds(j * 128, 128)])

            _loop(NP, last)

        @pl.when(it > 0)
        def _():
            _loop(NP - 1, lambda n: stage(n, STAGE_ORDER, _idle(0)))

        pl.when(it == 1)(x_copy(4, 4).wait)
        kb[:, pl.ds(0, HALO)] = ktail[pair]
        vb[:, pl.ds(0, HALO)] = vtail[pair]
        _run(LAST_ORDER, Q=a_scores(nxt, 0), R=a_scores(nxt, 1), v=a_values(nxt, NP - 1, 0),
             w=a_values(nxt, NP - 1, 1), u=a_update(NP - 1),
             P=a_out(0, _idle(0)),
             o=_chain(a_operands(NP - 2, 1), a_operands(NP - 1, 0), a_operands(NP - 1, 1)))
        fill = norm("xa", 0, HB, 8)
        _drain(a_out(1, fill))
        done(fill)
        for c in range(2):
            if c == 0:
                fill = _chain(norm("xa", 1, HB, 8), _spaced(gather(2, 1), 4, 4, 3))
            else:
                fill = _chain(_idle(12), _spaced(b_values(0), 1, 2, 2), _spaced(gather(3, 2), 3, 3, 4))
            b_proj(c, 0, fill)
            b_proj(c, 1, fill)
            done(fill)
            b_logits(c)
            fill = _chain(_idle(156), _spaced(b_probs(c), 2))
            b_proj(c, 2, fill)
            done(fill)
        fill = _chain(_idle(12), _spaced(b_values(1), 2, 1, 2, 2, 1))
        b_out(0, fill)
        done(fill)
        fill = norm("xb", 0, HA, 8)
        b_out(1, fill)
        done(fill)
        ktail[pair] = kb[:, pl.ds(L, HALO)]
        vtail[pair] = vb[:, pl.ds(L, HALO)]
        pl.when(pair == 1)(out_copy(2 * seg + 1, slice(None), pl.ds(D // 2, D // 2)).start)

    _loop(2 * NSEG, step)
    pltpu.make_async_copy(xout, out_hbm, sems.at[SEM_OUT]).wait()


@jax.jit
def pallas_interleave_layers__memory_aug_infini_attn__sliding_local_dilated__prompt_kernel(
    A_x, A_wq, A_wk, A_wv, A_wo, A_beta, B_x, B_wqkv, B_wo,
):
    del B_x
    hbm = pl.BlockSpec(memory_space=pl.ANY)
    vm = pltpu.VMEM
    chunks = (2 * NSEG, 2 * CH, D)
    heads = vm((1, 2, NCH, CH // 2, 128), I32)
    scratch = dict(
        ops=[vm((1, 8, CH // 2, D // 2), I32)] * 8,
        wb7=[vm((1, n, 7, D // 4, D // 2), I32) for n in (2, 1, 1)],
        tmp=vm((1, 4, G, H * PITCH + 32, 128), I32),
        park=[vm((1, CH, 128), F32)] * 2,
        stat=[vm((1, 2, 2 * CH, 128), F32)] * 2,
        xa=[vm((1, 2 * CH, D), F32)] * 2,
        xb=[vm((1, 2 * CH, D), F32)] * 2,
        nxt=dict(k=heads, qt=heads, vt=heads, pk=heads, pq=heads, z=vm((1, 2, NCH, 8, 128), F32)),
        cur=dict(k=heads, qt=heads, vt=heads),
        s=[[vm((1, (j + 1) * CH, 4 * CH), F32) for j in range(NCH)]] * 2,
        top=[[vm((1, 16, 4 * CH), F32)] * NCH] * 2,
        r=[vm((1, 136, L), F32)] * 2,
        ot=[vm((1, 2, 2, 128, CH), F32)] * 2,
        qb=[vm((1, G + 4, 2 * CH + 8, 128), F32)] * 2,
        lb=[vm((1, WIN, 2 * CH + 8, 128), F32)] * 2,
        kb=vm((1, G, HALO + L + 24, 128), F32),
        vb=vm((1, G, HALO + L + 24, 128), F32),
    )
    out = pl.pallas_call(
        _kernel,
        name="infini_dilated",
        out_shape=jax.ShapeDtypeStruct(chunks, BF16),
        in_specs=[hbm] * 8,
        out_specs=hbm,
        scratch_shapes=[
            vm(chunks, BF16), vm(chunks, BF16),
            vm((NP + 2, 3, D, 256), BF16), vm((3, D, D), BF16), vm((D, D), BF16),
            [vm((NP + 1 + (m == 0), 7, D // 4, 128), I32) for m in range(3)],
            vm((2, NP, 2, 144, 128), F32), vm((NP, 8, 128), F32), vm((DH, CH), F32),
            vm((2, G, HALO, 128), F32), vm((2, G, HALO, 128), F32),
            scratch, pltpu.SMEM((NP,), I32), pltpu.SemaphoreType.DMA((SEM_OUT + 1,)), vm((H,), BF16),
        ],
        compiler_params=pltpu.CompilerParams(vmem_limit_bytes=110 * 2 ** 20),
    )(A_x.reshape(chunks), A_wq, A_wk, A_wv, A_wo, A_beta, B_wqkv, B_wo)
    return out.reshape(A_x.shape)
```

```python
import math

import jax
import jax.numpy as jnp
from jax import lax
import jax.experimental.pallas as pl
import jax.experimental.pallas.tpu as pltpu

S = 2048
D = 1024
H = 32
DH = D // H
NSEG = 4
L = S // NSEG
WIN, DIL = 8, 2
HALO = 16
G = D // 128
NP = G // 2
CH = 128
NCH = L // CH
PITCH = DH // 2 + 1
QSCALE = DH ** -0.5 * math.log2(math.e)
NEG = -1e9
HA, OA, HB, OB = 0, 2, 4, 6
SEM_BETA, SEM_WB, SEM_PANEL, SEM_WOB, SEM_OUT = 3, 5, 8, 16, 17

STAGE_ORDER = "PPQPPPQQQPPvPPvPvPvvPPvQvvPvvPvPQPQPPvvPPvQvvvPPvvPvPvPPPvPvPvPvPrvPvvPvvPvPPvvPPPvrPP"
FIRST_ORDER = "PPQPQPQPQPPvPPvPvPvPvPQvvPvQPPvvQvPPvPQvPPvvPvPvPvPvPvPvPvPPvvPvPrvPvPvvvPPvPPvPvPvPPr"
LAST_ORDER = "ooooQQRRvvQwvwvwRwvwooooQRPvPvPvvPvPPvPvvPPvPPvPvvPvwPwPwwwPwwPwPPwwPwPwPwPPPPPPoooo"

F32, BF16, I32 = jnp.float32, jnp.bfloat16, jnp.int32
NN = (((1,), (0,)), ((), ()))
NT = (((1,), (1,)), ((), ()))


def _dot(a, b, dims=NN):
    return lax.dot_general(a, b, dims, preferred_element_type=F32)


def _pack(x):
    return pltpu.bitcast(x.astype(BF16), I32)


def _unpack(x):
    return pltpu.bitcast(x, BF16)


def _cat(xs, axis):
    return xs[0] if len(xs) == 1 else lax.concatenate(xs, axis)


def _tree(fn, xs):
    while len(xs) > 1:
        xs = [fn(xs[i], xs[i + 1]) if i + 1 < len(xs) else xs[i] for i in range(0, len(xs), 2)]
    return xs[0]


def _cols(x):
    return [x[:, g * 128:(g + 1) * 128] for g in range(x.shape[1] // 128)]


def _fold(fn, x):
    return fn(x.reshape(x.shape[0] // 8, 8, x.shape[1]), axis=0)


def _digest(x, rows=8):
    for n in (4 * rows, 2 * rows, rows):
        x = x[:n] | x[-n:]
    return x


def _iota(shape, dim):
    return lax.broadcasted_iota(I32, shape, dim)


def _aligned(i, n):
    return i if isinstance(i, int) else pl.multiple_of(i, n)


def _loop(n, body):
    def trip(i, carry):
        body(i)

    lax.fori_loop(0, n, trip, None)


def _row_mean(x):
    c = _cols(x)
    return _tree(lax.add, [jnp.sum(c[i] + c[i + 4], axis=-1, keepdims=True) for i in range(4)]) * (1.0 / D)


def _phi(t):
    return jnp.maximum(t, 0.0) + jnp.exp(jnp.minimum(t, 0.0))


def _rcp(x):
    return pltpu.reciprocal(x, approx=False, full_range=False)


def _rotate_quarters(xs, sign):
    for bit in (1, 2):
        on = _iota(xs[0].shape, 1) & (DH * bit) != 0
        xs = [lax.select(on, xs[(i + sign * bit) % 4], xs[i]) for i in range(4)]
    return xs


def _shift_rows(x, j):
    n = x.shape[0] // 4 * (j % 4)
    return _cat([x[n:], x[:n]], 0) if n else x


def _pick(r, x, y=None):
    n = x.shape[0] // 4
    lane = _iota((n, 128), 1) & (3 * DH)
    return _cat([lax.select(lane == (a + r) % 4 * DH, x[a * n:(a + 1) * n],
                            jnp.zeros((n, 128), x.dtype) if y is None else y[a * n:(a + 1) * n]) for a in range(4)], 0)


def _rotate_rows(x, sign):
    n = x.shape[0] // 4
    return _cat(_rotate_quarters([x[i * n:(i + 1) * n] for i in range(4)], sign), 0)


def _exchange(xs, j):
    ys = _rotate_quarters(xs, 1)
    return [ys[(-i - j) % 4] for i in range(4)]


def _lhs7(block, put):
    a11 = block(0, 0)
    yield put((2, a11))
    a22 = block(1, 1)
    yield put((3, a22), (0, a11 + a22))
    a12 = block(0, 1)
    yield put((4, a11 + a12), (6, a12 - a22))
    a21 = block(1, 0)
    yield put((1, a21 + a22), (5, a21 - a11))


def _rhs7(b11, b12, b21, b22):
    return [b11 + b22, b11, b12 - b22, b21 - b11, b22, b11 + b12, b21 + b22]


def _strassen(prod, emit, park):
    m6 = prod(5)
    yield
    m2 = prod(1)
    park[0][...] = m6 - m2
    yield
    m4 = prod(3)
    emit(1, 0, m2 + m4)
    yield
    m1 = prod(0)
    c22 = park[0][...] + m1
    park[1][...] = m4 + m1
    yield
    m3 = prod(2)
    emit(1, 1, c22 + m3)
    yield
    m5 = prod(4)
    emit(0, 1, m3 + m5)
    c11 = park[1][...] - m5
    yield
    emit(0, 0, c11 + prod(6))
    yield


def _chain(*gens):
    for g in gens:
        yield from g


def _idle(n):
    for _ in range(n):
        yield


def _spaced(gen, *gaps):
    for i, x in enumerate(gen):
        yield x
        yield from _idle(gaps[i % len(gaps)] - 1)


def _merge(a, b):
    while True:
        xs = [x for x in (next(a, _merge), next(b, _merge)) if x is not _merge]
        if not xs:
            return
        xs = [x for x in xs if x is not None]
        yield _tree(lax.bitwise_or, xs) if xs else None


def _drain(gen):
    for _ in gen:
        pass


def _run(order, **gens):
    for ch in order.replace(" ", ""):
        next(gens[ch])
    for name, g in gens.items():
        assert next(g, _run) is _run, name


class _Buf:
    def __init__(self, ref, z):
        self.ref, self.z = ref, z

    def __setitem__(self, idx, val):
        self.ref[(0,) + (idx if isinstance(idx, tuple) else (idx,))] = val

    def __getitem__(self, idx):
        return self.ref[(self.z,) + (idx if isinstance(idx, tuple) else (idx,))]


def _kernel(x_hbm, wq_hbm, wk_hbm, wv_hbm, wo_hbm, beta_hbm, wqkv_hbm, wob_hbm, out_hbm,
            xin, xout, wa_raw, wqkv_raw, wob_raw, wa7, mem, gate, bias, ktail, vtail, scratch, zero, sems, beta):
    def panel_copy(m, n):
        src, col = ((wk_hbm, wq_hbm, wv_hbm)[m], n) if n < NP else (wo_hbm, 3 * (n - NP) + m)
        return pltpu.make_async_copy(src.at[:, pl.ds(col * 256, 256)], wa_raw.at[n, m],
                                     sems.at[SEM_PANEL + (2 + n if n else m)])

    def x_copy(i, n=1):
        return pltpu.make_async_copy(x_hbm.at[pl.ds(i, n)], xin.at[pl.ds(i, n)], sems.at[i])

    def wb_copy(m):
        return pltpu.make_async_copy(wqkv_hbm.at[:, pl.ds(_aligned(m * D, D), D)], wqkv_raw.at[m],
                                     sems.at[SEM_WB + m])

    def out_copy(*at):
        return pltpu.make_async_copy(xout.at[at], out_hbm.at[at], sems.at[SEM_OUT])

    beta_copy = pltpu.make_async_copy(beta_hbm, beta, sems.at[SEM_BETA])
    beta_copy.start()
    x_copy(0).start()
    for n in range(NP + 1):
        if n >= 2:
            wb_copy(n - 2).start()
        for m in range(3):
            panel_copy(m, n).start()
            if (m, n) == (1, 0):
                x_copy(1).start()
    last_copies = [panel_copy(0, NP + 1), pltpu.make_async_copy(wob_hbm, wob_raw, sems.at[SEM_WOB]),
                   x_copy(2, 2)]
    for c in last_copies:
        c.start()
    x_copy(4, 4).start()

    def clear(i):
        zero[i] = 0
        mem[:, i] = jnp.zeros((2,) + mem.shape[2:], F32)
        for tail in (ktail, vtail):
            tail[:, pl.ds(2 * i, 2)] = jnp.zeros((2, 2, HALO, 128), F32)
        scratch["tmp"][0, 0, pl.ds(2 * i, 2)] = jnp.zeros((2, H * PITCH + 32, 128), I32)
        scratch["ot"][1][0, i // 2, i % 2] = jnp.zeros((128, CH), F32)

    _loop(NP, clear)
    z = zero[1]
    st = jax.tree.map(lambda r: _Buf(r, z), scratch)
    ops, wb7, tmp, nxt, cur, qb, kb, vb = [st[k] for k in ("ops", "wb7", "tmp", "nxt", "cur", "qb", "kb", "vb")]

    def prep_rows(m, n, k):
        rows = [pl.ds(_aligned((2 * k + r) * CH, CH), CH) for r in range(2)]
        ws = _rhs7(*[w for r in rows for w in _cols(wa_raw[n, m, r, :].astype(F32))])
        out = _cols(_pack(_cat([ws[j] for j in (0, 2, 3, 5, 6)], 1)))
        out += [_pack(wa_raw[n + z, m, rows[r], pl.ds(r * 128, 128)]) for r in range(2)]
        for j, w in zip((0, 2, 3, 5, 6, 1, 4), out):
            wa7[m][n, j, pl.ds(_aligned(k * (CH // 2), CH // 2), CH // 2), :] = w
        return out

    def prep_panel(m, n):
        for k in range(NP):
            bits = _tree(lax.bitwise_or, prep_rows(m, n, k))
            for b in range(CH // 16):
                yield bits[8 * b:8 * b + 8]

    def wait_panels(n):
        pltpu.make_async_copy(wa_raw.at[n], wa_raw.at[n], sems.at[SEM_PANEL + 2 + n]).wait()

    def spread(m, j, g, w):
        w = _pack(w)
        for h in range(8):
            tmp[m, j, pl.ds((8 * g + h) * PITCH, DH // 2)] = w[h * DH // 2:(h + 1) * DH // 2]
        return w[-8:]

    def spread_qkv(m):
        for j in range(G):
            for g in range(NP):
                yield spread(m, j, g, wqkv_raw[m, pl.ds(j * 128, 128), pl.ds(g * 256, 256)].T)

    def gather(m, dst, slot=0):
        for k in range(2 * NP):
            ws = [_cat([tmp[m, j, pl.ds(k // 2 * 4 + k % 2 + 2 * r, H, stride=PITCH)] for j in range(s, G, 2)], 1)
                  for r in range(2) for s in range(2)]
            a, b, c, d = [lax.bitcast_convert_type(_cat([w << 16, w & -65536], 0), F32) for w in ws]
            ws = _pack(_cat(_rhs7(a, c, b, d) if dst < 2 else _rhs7(a, b, c, d), 0))
            wb7[dst][slot, :, pl.ds(k * H, H)] = ws.reshape(7, H, D // 2)
            bits = _cols(_digest(ws, H))
            for half in (bits[0] | bits[1], bits[2] | bits[3]):
                for row in (0, 16, 8, 24):
                    yield half[row:row + 8]

    recent, pending = [], []

    def streamed(y, slots=None):
        recent.extend((y, 16 * b) for b in range(slots or y.shape[0] // 16))

    def result(age):
        y, row = recent[-age]
        return y[row:row + 8, :128]

    def project(slot, rhs, emit, fill, dims=NN):
        def prod(i):
            rows, start = [], 0
            for b in range(CH // 16):
                mark = next(fill, None)
                while b == 0 and pending and pending[0][0] <= len(recent):
                    late = pending.pop(0)[1]
                    mark = late if mark is None else mark | late
                if mark is None:
                    continue
                if len(recent) >= 12 - b:
                    mark = mark | lax.bitcast_convert_type(result(12 - b), I32)
                if b > start:
                    rows.append(ops[slot][i, pl.ds(8 * start, 8 * (b - start))])
                    start = b
                ops[slot][7, pl.ds(8 * b, 8), pl.ds(0, 128)] = mark
            rows.append(ops[slot][i, pl.ds(8 * start, CH // 2 - 8 * start)])
            y = _dot(_unpack(_cat(rows, 0)), _unpack(rhs(i)), dims)
            streamed(y)
            return y

        return _strassen(prod, emit, st["park"])

    def done(fill):
        assert next(fill, done) is done
        recent.clear()
        pending.clear()

    def put_operand(slot, b, n):
        def put(*items):
            packed = _cols(_pack(_cat([a for _, a in items], 1)))
            for (i, _), a in zip(items, packed):
                ops[slot][i, pl.ds(8 * b, 8), pl.ds(n * 128, 128)] = a
            return _tree(lax.bitwise_or, packed)

        return put

    def put_chunk(slot, h):
        h, parts = _cols(h), []
        _drain(_lhs7(lambda r, s: _cat(h[s::2], 1)[r * CH:(r + 1) * CH], lambda *items: parts.extend(items)))
        packed = _pack(_cat([a for _, a in sorted(parts, key=lambda item: item[0])], 0))
        ops[slot][pl.ds(0, 7)] = packed.reshape(7, CH // 2, D // 2)
        return packed

    def norm(x, c, slot, gap):
        x, stat = st[x][c], st["stat"][c]
        for b in range(2 * CH // 16):
            rows = pl.ds(16 * b, 16)
            v = x[rows]
            m = _row_mean(v)
            d = v - m
            stat[0, rows] = jnp.broadcast_to(m, (16, 128))
            stat[1, rows] = jnp.broadcast_to(lax.rsqrt(_row_mean(d * d) + 1e-5), (16, 128))

        def apply():
            h = (x[...] - _cat([stat[0]] * G, 1)) * _cat([stat[1]] * G, 1)
            bits = _cols(_digest(put_chunk(slot + c, h), CH // 2))
            bits = [bits[0] | bits[1], bits[2] | bits[3]]
            for b in range(CH // 16):
                for half in bits:
                    yield half[8 * b:8 * b + 8]

        return _chain(_idle(72), _spaced(apply(), gap))

    bias[...] = jnp.where(_iota((DH, CH), 0) > _iota((DH, CH), 1) % DH, NEG, 0.0)
    beta_copy.wait()
    b = jnp.broadcast_to(beta[...].astype(F32).reshape(1, H), (H, H))
    b = jnp.sum(jnp.where(_iota((H, H), 0) == _iota((H, H), 1), b, 0.0), axis=1, keepdims=True)
    gate[...] = jnp.broadcast_to(1.0 / (1.0 + jnp.exp(-b)), (H, 128)).reshape(NP, 8, 128)
    x_copy(0).wait()
    x = xin[0].astype(F32)
    st["xb"][0][...] = x
    d = x - jnp.mean(x, axis=-1, keepdims=True)
    put_chunk(HA, d * lax.rsqrt(jnp.mean(d * d, axis=-1, keepdims=True) + 1e-5))
    for m in range(3):
        panel_copy(m, 0).wait()
        _loop(NP, lambda k: prep_rows(m, 0, k))
        if m == 1:
            x_copy(1).wait()
            st["xb"][1][...] = xin[1].astype(F32)

    def step(it):
        seg, pair = it // 2, it % 2

        def a_proj(m, n, c, fill):
            def emit(r, e, y):
                j = 2 * c + r
                if m == 0:
                    pk = _phi(y)
                    nxt["k"][e, j], nxt["pk"][e, j] = _cols(_pack(_cat([y, pk], 1)))
                    nxt["z"][e, j] = _fold(jnp.sum, pk)
                    return
                if m == 1:
                    y = _rotate_rows(_shift_rows(y, -j), -1)
                    nxt["pq"][e, j] = _pack(_phi(y))
                    y = y * QSCALE
                else:
                    st["v0"][e, pl.ds(j * DH, DH)] = y[:DH]
                y = _pack(y.astype(BF16).T)
                nxt["qt" if m == 1 else "vt"][e, j] = y
                pending.append((len(recent) + 40, y[-8:]))

            return project(HA + c, lambda i: wa7[m][n, i], emit, fill)

        def a_recall(n):
            for e in range(2):
                r = _dot(mem[pair, n, e].astype(BF16), _unpack(nxt["pq"][e].reshape(L // 2, 128)), NT)
                st["r"][e][...] = r[:136]
                yield

        def a_first_values():
            for e in range(2):
                w = _pack(st["v0"][e].astype(BF16).T)
                nxt["v0"][e, 0] = w
                yield w[-8:]

        def a_count(n):
            own = _iota((16, 128), 0) == _iota((16, 128), 1) // DH
            for e in range(2):
                zs = jnp.sum(jnp.sum(nxt["z"][e], axis=0), axis=0, keepdims=True)
                zs = mem[pair, n, e, pl.ds(128, 16)] + jnp.where(own, zs, 0.0)
                mem[pair, n, e, pl.ds(128, 16)] = zs
                yield lax.bitcast_convert_type(zs[:8], I32)

        def a_scores(src, e):
            blank = jnp.zeros((DH // 2, CH), I32)
            for j in range(NCH):
                qt = src["qt"][e, j]
                top = [None] * 4
                for t in reversed(range(4)):
                    sc = _dot(_unpack(src["k"][e, j, pl.ds(0, (t + 1) * DH // 2)]),
                              _unpack(_pick(t + j, qt)))
                    sc = _cat([sc[:t * DH]] * (t > 0) + [sc[t * DH:] + bias[...]], 0)
                    st["s"][e][j][pl.ds(j * CH, (t + 1) * DH), pl.ds(t * CH, CH)] = sc
                    top[t] = _fold(jnp.max, sc)
                    if t == 3:
                        streamed(sc, 5)
                top = _cat(_exchange(top, j), 1)
                if j > 0:
                    heads = [_cat([qt[a * DH // 2:(a + 1) * DH // 2] if a == hh else blank for a in range(4)], 0)
                             for hh in range(4)]
                    sc = _dot(_unpack(src["k"][e, pl.ds(0, j)].reshape(j * CH // 2, 128)), _unpack(_cat(heads, 1)))
                    st["s"][e][j][pl.ds(0, j * CH)] = sc
                    top = jnp.maximum(top, _fold(jnp.max, sc))
                    streamed(sc)
                st["top"][e][j][pl.ds(0, 8)] = jnp.broadcast_to(jnp.max(top, axis=0, keepdims=True), (8, 4 * CH))
                yield

        def a_values(src, n, e, span):
            def tops(j):
                if len(recent) >= 17:
                    st["top"][e][j][pl.ds(8, 8), pl.ds(0, 128)] = result(17)
                return _cols(st["top"][e][j][pl.ds(0, 8)])

            def probs(j, row, rows, col, top):
                p = jnp.exp2(st["s"][e][j][pl.ds(row, rows), pl.ds(col * CH, CH)] - _cat([top] * (rows // 8), 0))
                l = p[-16:]
                for a in reversed(range(rows // 16 - 1)):
                    l = l + p[16 * a:16 * a + 16]
                return p, _fold(jnp.sum, l)

            def mix(i, hh, p):
                return _dot(_unpack(src["vt"][e, i, pl.ds(hh * DH // 2, DH // 2)]), p.astype(BF16))

            def finish(j, hh, acc, l):
                g = gate[n, pl.ds(4 * e + hh, 1), :]
                rden = _rcp(st["r"][e][pl.ds(128 + hh, 1), pl.ds(j * CH, CH)] + 1e-6)
                rl = _rcp(jnp.sum(l, axis=0, keepdims=True))
                st["ot"][j // 2][j % 2, e, pl.ds(hh * DH, DH)] = (
                    acc * ((1.0 - g) * rl) + st["r"][e][pl.ds(hh * DH, DH), pl.ds(j * CH, CH)] * (g * rden))

            side = st["side"][e]
            for j in range(NCH):
                if j % span == 0:
                    p, l = zip(*[probs(i, i * CH, DH, 0, _exchange(tops(i), i)[0]) for i in range(j, j + span)])
                    blank = [jnp.zeros((DH // 2, CH), I32)]
                    p = _cat(blank * j + [_pack(_cat(p, 0))] + blank * (NCH - j - span), 0)
                    o = _cat([_dot(_unpack(src["v0"][e, 0, pl.ds(hh * DH // 2, DH // 2)]),
                                   _unpack(_pick(hh, p))) for hh in range(4)], 0)
                    side[...] = side[...] + o if j else o
                    st["lsum"][e][pl.ds(8 * j, 8 * span)] = _cat(l, 0)
                    yield
                p, l = zip(*[probs(j, j * CH, (t + 1) * DH, t, top)
                             for t, top in enumerate(_exchange(tops(j), j)) if t])
                l = _exchange([st["lsum"][e][pl.ds(8 * j, 8)], *l], j)
                pk = cur["pk"][e, j]
                p = [_exchange([pk[a * DH // 2:(a + 1) * DH // 2]] + [jnp.zeros((DH // 2, CH), I32)] * max(a - 1, 0)
                               + _cols(_pack(_cat([w[a * DH:(a + 1) * DH] for w in p[max(a - 1, 0):]], 1))), j)
                     for a in range(4)]
                o = _cat([mix(j, hh, _unpack(_cat([p[a][hh] for a in range(4)], 0))) for hh in range(4)], 0)
                held = side[...]
                o, held = _pick(j, held, o), _pick(j, o, held)
                if j < NCH - 1:
                    side[...] = held
                else:
                    held = (held + pltpu.roll(held, 64, 1)) + (pltpu.roll(held, 32, 1) + pltpu.roll(held, 96, 1))
                    held = mem[pair, n, e, pl.ds(0, 128)] + _pick(0, held)
                    mem[pair, n, e, pl.ds(0, 128)] = held
                    pending.append((len(recent) + 32, lax.bitcast_convert_type(_fold(jnp.max, held), I32)))
                acc = [o[hh * DH:(hh + 1) * DH] for hh in range(4)]
                if j == 0:
                    for hh in range(4):
                        finish(j, hh, acc[hh], l[hh])
                yield
                for hp in range(2):
                    for i in range(j):
                        top = tops(j)
                        for hh in (2 * hp, 2 * hp + 1):
                            p, more = probs(j, i * CH, CH, hh, top[hh])
                            acc[hh], l[hh] = acc[hh] + mix(i, hh, p), l[hh] + more
                            if i == j - 1:
                                finish(j, hh, acc[hh], l[hh])
                        yield

        def a_operands(n, c):
            col = _aligned(n * 128, 128)

            def put(*items):
                out = [_rotate_rows(_pack(a.astype(BF16).T), 1) for _, a in items]
                for (i, _), a in zip(items, out):
                    ops[OA + c][i, :, pl.ds(col, 128)] = a
                return _tree(lax.bitwise_or, [a[-8:] for a in out])

            return _lhs7(lambda r, e: st["ot"][c][r, e], put)

        def a_out(c, fill):
            for n in range(NP):
                def emit(r, s, y):
                    at = (pl.ds(r * CH, CH), pl.ds((2 * n + s) * 128, 128))
                    st["xa"][c][at] = st["xb"][c][at] + _shift_rows(y, 2 * c + r)

                yield from project(OA + c, lambda i: wa7[n % 3][NP + n // 3, i], emit, fill)

        def b_proj(c, m, fill):
            for n in range(NP):
                def emit(r, s, y):
                    if m == 0:
                        qb[c][2 * n + s, pl.ds(r * CH, CH)] = y * QSCALE
                    else:
                        (kb, vb)[m - 1][2 * n + s, pl.ds(HALO + (2 * c + r) * CH, CH)] = y

                _drain(project(HB + c, lambda i: wb7[m // 2][m % 2, i, pl.ds(n * CH // 2, CH // 2)], emit, fill, NT))

        def b_logits(c):
            for b in range(2 * CH // 16):
                t0 = 2 * c * CH + 16 * b
                q = qb[c][pl.ds(0, G), pl.ds(16 * b, 16)]
                for w in range(WIN):
                    a = jnp.sum(q * kb[:, pl.ds(HALO + t0 - DIL * w, 16)], axis=0)
                    a = (a + pltpu.roll(a, 64, 1)) + (pltpu.roll(a, 32, 1) + pltpu.roll(a, 96, 1))
                    if t0 < DIL * w:
                        a = jnp.where(_iota((16, 128), 0) + (seg * L + t0) >= DIL * w, a, NEG)
                    st["lb"][c][w, pl.ds(16 * b, 16)] = a

        def b_probs(c):
            a = st["lb"][c][:, pl.ds(0, 2 * CH)]
            p = jnp.exp2(a - jnp.max(a, axis=0, keepdims=True))
            qb[c][pl.ds(0, WIN), pl.ds(0, 2 * CH)] = p
            l = jnp.sum(p, axis=0)
            st["stat"][c][0] = _rcp(l)
            l = lax.bitcast_convert_type(l, I32)
            for b in range(2 * CH // 8):
                yield l[8 * b:8 * b + 8]

        def b_values(c):
            for b in range(CH // 16):
                for n in range(NP):
                    if len(recent) >= 16:
                        qb[c][WIN, pl.ds(0, 8)] = result(16)
                    o = []
                    for r in range(2):
                        rows = pl.ds(r * CH + 16 * b, 16)
                        t0 = HALO + (2 * c + r) * CH + 16 * b
                        v = _cat([vb[pl.ds(2 * n, 2), pl.ds(t0 - DIL * w, 16)] for w in range(WIN)], 1)
                        a = v.reshape(2, WIN, 16, 128) * qb[c][pl.ds(0, WIN), rows]
                        o.append(jnp.sum(a, axis=1) * st["stat"][c][0, rows])
                    yield from _lhs7(lambda r, s: o[r][s], put_operand(OB + c, b, n))

        def b_out(c, fill):
            following = 2 * jnp.minimum(seg + 1, NSEG - 1) + c
            for n in range(NP):
                def emit(r, s, y):
                    at = (pl.ds(r * CH, CH), pl.ds((2 * n + s) * 128, 128))
                    x = st["xa"][c][at] + y
                    xout[(2 * seg + c,) + at] = x.astype(BF16)
                    st["xb"][c][at] = jnp.where(pair == 1, xin[(following,) + at].astype(F32), x)

                for i, _ in enumerate(project(OB + c, lambda i: wb7[2][0, i, :, pl.ds(n * 128, 128)], emit, fill)):
                    if (c, n, i) == (1, 2, 1):
                        @pl.when(pair == 1)
                        def _():
                            out_copy(2 * seg).start()
                            out_copy(2 * seg + 1, slice(None), pl.ds(0, D // 2)).start()

        for c in range(2):
            fill = _chain(_idle(96), a_first_values()) if c else norm("xb", 1, HA, 6)
            for m in (2, 1, 0):
                _drain(a_proj(m, 0, c, fill))
            done(fill)
        _drain(a_recall(0))

        def keep(name):
            for e in range(2):
                for j in range(nxt[name].ref.shape[2]):
                    w = nxt[name][e, j]
                    w = pltpu.roll(w, j * DH, 1) if name == "pk" and j else w
                    cur[name][e, j] = w
                    yield _digest(w)

        def stage(n, order, extra):
            fill = _merge(extra, _chain(
                keep("k"), keep("qt"), _merge(keep("vt"), keep("v0")), _merge(keep("pk"), a_count(n)),
                _spaced(a_operands(jnp.maximum(n - 1, 0), 1), 8), _idle(86), a_first_values(), _idle(120), _spaced(a_operands(n, 0), 8)))
            _run(order, P=_chain(*[a_proj(m, n + 1, c, fill) for m in (2, 1, 0) for c in range(2)]),
                 Q=_chain(a_scores(cur, 0), a_scores(cur, 1)), v=_chain(a_values(cur, n, 0, 4), a_values(cur, n, 1, 4)),
                 r=a_recall(n + 1))
            done(fill)

        def prepare(n):
            prev = jnp.maximum(n - 1, 0)
            yield from _spaced(gather(prev, 0, prev), 3, 3, 2)
            yield from _idle(5)
            wb_copy(n).wait()
            wait_panels(n + 2)
            yield from _merge(_chain(_idle(16), _spaced(spread_qkv(n), 4)),
                              _spaced(_chain(*[prep_panel(m, n + 2) for m in (0, 2, 1)]), 1, 2, 2))

        @pl.when(it == 0)
        def _():
            wait_panels(1)
            _loop(NP, lambda k: [prep_rows(m, 1, k) for m in range(3)])
            _loop(NP - 1, lambda n: stage(n, FIRST_ORDER, prepare(n)))
            for c in last_copies:
                c.wait()

            def last(k):
                prep_rows(0, NP + 1, k)
                for j in range(G):
                    spread(3, j, k, wob_raw[pl.ds(_aligned(k * 256, 256), 256), pl.ds(j * 128, 128)])

            _loop(NP, last)

        @pl.when(it > 0)
        def _():
            _loop(NP - 1, lambda n: stage(n, STAGE_ORDER, _idle(0)))

        pl.when(it == 1)(x_copy(4, 4).wait)
        kb[:, pl.ds(0, HALO)] = ktail[pair]
        vb[:, pl.ds(0, HALO)] = vtail[pair]
        _drain(_chain(keep("pk"), a_count(NP - 1)))
        _run(LAST_ORDER, Q=a_scores(nxt, 0), R=a_scores(nxt, 1), v=a_values(nxt, NP - 1, 0, 2),
             w=a_values(nxt, NP - 1, 1, 2),
             P=a_out(0, _idle(0)),
             o=_chain(a_operands(NP - 2, 1), a_operands(NP - 1, 0), a_operands(NP - 1, 1)))
        fill = norm("xa", 0, HB, 8)
        _drain(a_out(1, fill))
        done(fill)
        for c in range(2):
            if c == 0:
                fill = _chain(norm("xa", 1, HB, 8), _spaced(gather(2, 1), 4, 4, 3))
            else:
                fill = _chain(_idle(12), _spaced(b_values(0), 1, 2, 2), _spaced(gather(3, 2), 3, 3, 4))
            b_proj(c, 0, fill)
            b_proj(c, 1, fill)
            done(fill)
            b_logits(c)
            fill = _chain(_idle(156), _spaced(b_probs(c), 2))
            b_proj(c, 2, fill)
            done(fill)
        fill = _chain(_idle(12), _spaced(b_values(1), 2, 1, 2, 2, 1))
        b_out(0, fill)
        done(fill)
        fill = norm("xb", 0, HA, 8)
        b_out(1, fill)
        done(fill)
        ktail[pair] = kb[:, pl.ds(L, HALO)]
        vtail[pair] = vb[:, pl.ds(L, HALO)]
        pl.when(pair == 1)(out_copy(2 * seg + 1, slice(None), pl.ds(D // 2, D // 2)).start)

    _loop(2 * NSEG, step)
    pltpu.make_async_copy(xout, out_hbm, sems.at[SEM_OUT]).wait()


@jax.jit
def pallas_interleave_layers__memory_aug_infini_attn__sliding_local_dilated__prompt_kernel(
    A_x, A_wq, A_wk, A_wv, A_wo, A_beta, B_x, B_wqkv, B_wo,
):
    del B_x
    hbm = pl.BlockSpec(memory_space=pl.ANY)
    vm = pltpu.VMEM
    chunks = (2 * NSEG, 2 * CH, D)
    heads = vm((1, 2, NCH, CH // 2, 128), I32)
    scratch = dict(
        ops=[vm((1, 8, CH // 2, D // 2), I32)] * 8,
        wb7=[vm((1, n, 7, D // 4, D // 2), I32) for n in (2, 1, 1)],
        tmp=vm((1, 4, G, H * PITCH + 32, 128), I32),
        park=[vm((1, CH, 128), F32)] * 2,
        stat=[vm((1, 2, 2 * CH, 128), F32)] * 2,
        xa=[vm((1, 2 * CH, D), F32)] * 2,
        xb=[vm((1, 2 * CH, D), F32)] * 2,
        nxt=dict(k=heads, qt=heads, vt=heads, pk=heads, pq=heads, z=vm((1, 2, NCH, 8, 128), F32),
                 v0=vm((1, 2, 1, CH // 2, 128), I32)),
        v0=vm((1, 2, CH, 128), F32),
        cur=dict(k=heads, qt=heads, vt=heads, pk=heads, v0=vm((1, 2, 1, CH // 2, 128), I32)),
        side=[vm((1, 128, CH), F32)] * 2,
        lsum=[vm((1, 32, CH), F32)] * 2,
        s=[[vm((1, (j + 1) * CH, 4 * CH), F32) for j in range(NCH)]] * 2,
        top=[[vm((1, 16, 4 * CH), F32)] * NCH] * 2,
        r=[vm((1, 136, L), F32)] * 2,
        ot=[vm((1, 2, 2, 128, CH), F32)] * 2,
        qb=[vm((1, G + 4, 2 * CH + 8, 128), F32)] * 2,
        lb=[vm((1, WIN, 2 * CH + 8, 128), F32)] * 2,
        kb=vm((1, G, HALO + L + 24, 128), F32),
        vb=vm((1, G, HALO + L + 24, 128), F32),
    )
    out = pl.pallas_call(
        _kernel,
        name="infini_dilated",
        out_shape=jax.ShapeDtypeStruct(chunks, BF16),
        in_specs=[hbm] * 8,
        out_specs=hbm,
        scratch_shapes=[
            vm(chunks, BF16), vm(chunks, BF16),
            vm((NP + 2, 3, D, 256), BF16), vm((3, D, D), BF16), vm((D, D), BF16),
            [vm((NP + 1 + (m == 0), 7, D // 4, 128), I32) for m in range(3)],
            vm((2, NP, 2, 144, 128), F32), vm((NP, 8, 128), F32), vm((DH, CH), F32),
            vm((2, G, HALO, 128), F32), vm((2, G, HALO, 128), F32),
            scratch, pltpu.SMEM((NP,), I32), pltpu.SemaphoreType.DMA((SEM_OUT + 1,)), vm((H,), BF16),
        ],
        compiler_params=pltpu.CompilerParams(vmem_limit_bytes=110 * 2 ** 20),
    )(A_x.reshape(chunks), A_wq, A_wk, A_wv, A_wo, A_beta, B_wqkv, B_wo)
    return out.reshape(A_x.shape)
```
